```python
import jax
import jax.numpy as jnp

def _softmax(x, axis=-1):
    return jax.nn.softmax(x, axis=axis)
def _gelu(x):
    return jax.nn.gelu(x, approximate=True)
def _silu(x):
    return jax.nn.silu(x)
def _sigmoid(x):
    return jax.nn.sigmoid(x)
def _layernorm(x, axis=-1, eps=1e-5):
    m = jnp.mean(x, axis=axis, keepdims=True)
    v = jnp.var(x, axis=axis, keepdims=True)
    return (x - m) / jnp.sqrt(v + eps)
def _scatter_add(tgt, idx, src, axis=0):
    return tgt.at[idx].add(src)
def _segment_sum(src, seg, n):
    return jax.ops.segment_sum(src, seg, n)
class _Rng:
    def __init__(self, key):
        self._k = key
    def _next(self):
        self._k, sub = jax.random.split(self._k)
        return sub
    def normal(self, shape):
        return jax.random.normal(self._next(), shape, dtype=jnp.bfloat16)
    def randint(self, lo, hi, shape):
        return jax.random.randint(self._next(), shape, lo, hi, dtype=jnp.int32)
    def uniform(self, shape, lo=0.0, hi=1.0):
        return jax.random.uniform(self._next(), shape, jnp.bfloat16, lo, hi)
    def permutation(self, n):
        return jax.random.permutation(self._next(), n)


kernel_name = 'gated_mix__mha_block_cached__moe_arch_mod__decode'

def setup_inputs():
    _rng = _Rng(jax.random.key(int.from_bytes(__import__("os").urandom(4), "little")))
    _w = (lambda a: (lambda t: t.astype(jnp.bfloat16) if jnp.issubdtype(t.dtype, jnp.floating) else t)(jnp.asarray(a)))
    def _A_setup():
        B, Sq, D = 4, 1, 1024
        H, Sk, Dh = 32, 8192, 128
        return {
            "x": _w((lambda *s: _rng.normal(s) * 0.05)(B, Sq, D)),
            "k_cache": _w((lambda *s: _rng.normal(s) * 0.05)(B, H, Sk, Dh)),
            "v_cache": _w((lambda *s: _rng.normal(s) * 0.05)(B, H, Sk, Dh)),
            "wq": _w((lambda *s: _rng.normal(s) * 0.05)(D, H * Dh) * (D ** -0.5)),
            "wo": _w((lambda *s: _rng.normal(s) * 0.05)(H * Dh, D) * ((H * Dh) ** -0.5)),
        }
    _A_in = _A_setup()

    def _B_setup():
        B, S, D, F, C = 4, 1, 1024, 3584, 1
        return {
            "x": _w((lambda *s: _rng.normal(s) * 0.05)(B, S, D)),
            "w_r": _w((lambda *s: _rng.normal(s) * 0.05)(D)),
            "w_gate": _w((lambda *s: _rng.normal(s) * 0.05)(D, F)),
            "w_up": _w((lambda *s: _rng.normal(s) * 0.05)(D, F)),
            "w_down": _w((lambda *s: _rng.normal(s) * 0.05)(F, D)),
        }
    _B_in = _B_setup()

    return {
        "A_x": _A_in["x"],
        "A_k_cache": _A_in["k_cache"],
        "A_v_cache": _A_in["v_cache"],
        "A_wq": _A_in["wq"],
        "A_wo": _A_in["wo"],
        "B_x": _B_in["x"],
        "B_w_r": _B_in["w_r"],
        "B_w_gate": _B_in["w_gate"],
        "B_w_up": _B_in["w_up"],
        "B_w_down": _B_in["w_down"],
        "gate_w": _w((lambda *s: _rng.normal(s) * 0.05)(1024)),
    }

def reference(A_x, A_k_cache, A_v_cache, A_wq, A_wo, B_x, B_w_r, B_w_gate, B_w_up, B_w_down, gate_w):
    def _A_ref(x, k_cache, v_cache, wq, wo):
        B, Sq, D = x.shape
        H, Dh = 32, 128
        q = (lambda x, *d: x.transpose(*d))((x @ wq).reshape(B, Sq, H, Dh), 0, 2, 1, 3)
        scores = jnp.einsum("bhqd,bhkd->bhqk", q, k_cache) * (Dh ** -0.5)
        p = _softmax(scores, axis=-1)
        o = jnp.einsum("bhqk,bhkd->bhqd", p, v_cache)
        return (lambda x, *d: x.transpose(*d))(o, 0, 2, 1, 3).reshape(B, Sq, H * Dh) @ wo

    def _B_ref(x, w_r, w_gate, w_up, w_down):
        B, S, D = x.shape
        C = 1
        r = x @ w_r
        idx = jnp.argsort(-r, axis=-1)[:, :C]
        idx_e = jnp.repeat(idx.reshape(B, C, 1), D, axis=2)
        x_sel = jnp.take_along_axis(x, idx_e, axis=1)
        g = _silu(x_sel @ w_gate)
        u = x_sel @ w_up
        y = (g * u) @ w_down
        r_sel = _sigmoid(jnp.take_along_axis(r, idx, axis=1))
        y = y * r_sel.reshape(B, C, 1)
        b_off = (jnp.arange(B) * S).reshape(B, 1)
        flat_idx = (idx + b_off).reshape(B * C)
        zero = (x * 0.0).reshape(B * S, D)
        upd = _scatter_add(zero, flat_idx, y.reshape(B * C, D), axis=0)
        return x + upd.reshape(B, S, D)

    x = A_x
    g = _sigmoid((x * gate_w).sum(-1, keepdims=True))
    a = _A_ref(x, A_k_cache, A_v_cache, A_wq, A_wo)
    b = _B_ref(x, B_w_r, B_w_gate, B_w_up, B_w_down)
    return g * a + (1 - g) * b
```

```python
import jax
import jax.experimental.pallas as pl
import jax.experimental.pallas.tpu as pltpu
import jax.numpy as jnp
import numpy as np

B, D, H, SK, DH, F = 4, 1024, 32, 8192, 128, 3584

M = 8
PAGE = 32
BLOCK = 8
LEAD = 2
FAST = (4, 2)
NS = 16
HS = B * H // NS
KEYS = BLOCK * PAGE
OLD = LEAD * PAGE
JH = SK // KEYS
STEPS = HS * JH
DEPTH = 3
N_F = D * F // (KEYS * 128)
N_A = D * H * DH // (KEYS * 128)
SLAB = 128 * D // (KEYS * 128)
TAIL = 4
N_D = N_F - TAIL * SLAB
T_FFN = N_F + N_D + DEPTH
T_OUT = N_F + N_A + DEPTH
assert T_FFN + N_D // SLAB < STEPS and STEPS - JH <= T_OUT and T_OUT + HS < STEPS

F32, BF16 = jnp.float32, jnp.bfloat16
LOWEST = float(np.finfo(np.float32).min)


def _kernel(x_hbm, k_hbm, v_hbm, wq_hbm, wo_hbm, wr_hbm, wg_hbm, wu_hbm, wd_hbm, gw_hbm,
            out_ref,
            k_ring, v_ring, wq, wo, wg, wu, wd, x_in, wr, gw,
            xs, q_all, qs, run_max, run_sum, run_pv, p_old, p_new, act, y_acc, a_acc,
            k_sem, v_sem, w_sem, tail_sem, small_sem):

    def between(n, lo, hi):
        return jnp.logical_and(n >= lo, n < hi)

    def wait_all(buf, sem):
        pltpu.make_async_copy(buf, buf, sem).wait()

    def start_pages(src, dst, sem, fast=FAST[0]):
        for queue, rows in enumerate((pl.ds(0, fast), pl.ds(fast, PAGE - fast))):
            pltpu.make_async_copy(src.at[:, rows], dst.at[:, rows], sem).start(priority=queue)

    def for_streams(body):
        @pl.loop(0, NS // 2)
        def _(n):
            high = ((n & 1) << 3) + ((n & 2) << 1) + (n >> 2)
            for low in range(2):
                body(high + 2 * low, FAST[low])

    def start_weight(src, dst, sem, n, count, fast=FAST[0]):
        dst = dst.reshape(src.shape)

        @pl.when(n == 0)
        def _():
            for part in (pl.ds(count * BLOCK - LEAD, LEAD), pl.ds(0, BLOCK - LEAD)):
                start_pages(src.at[part], dst.at[part], sem, fast)

        @pl.when(between(n, 1, count))
        def _():
            part = pl.ds(n * BLOCK - LEAD, BLOCK)
            start_pages(src.at[part], dst.at[part], sem, fast)

    def start_first(src, ring, sem):
        def body(s, fast):
            prev = (s + NS - 1) % NS
            start_pages(src.at[pl.ds((prev + 1) * STEPS * BLOCK - LEAD, LEAD)],
                        ring.at[0, prev, pl.ds(0, LEAD)], sem.at[0], fast)
            start_pages(src.at[pl.ds(s * STEPS * BLOCK, BLOCK - LEAD)],
                        ring.at[0, s, pl.ds(LEAD, BLOCK - LEAD)], sem.at[0], fast)
        for_streams(body)

    def start_cache(src, ring, sem, j):
        slot = j % DEPTH
        for_streams(lambda s, fast: start_pages(
            src.at[pl.ds((s * STEPS + j) * BLOCK - LEAD, BLOCK)],
            ring.at[slot, s], sem.at[slot], fast))

    def times_tiles(lhs, w):
        return [jnp.dot(lhs, w[:, r:r + 8, :].reshape(-1, 128), preferred_element_type=F32)
                for r in range(0, PAGE, 8)]

    def times_slab(lhs, w, n):
        bands = pl.ds(n * 16, 16)
        return jnp.concatenate(
            times_tiles(lhs, w[bands, 0]) + times_tiles(lhs, w[bands, 1]), axis=1)

    def per_stream(lhs, fn):
        halves = []
        for row0 in range(0, NS, M):
            part = lhs[row0:row0 + M].astype(BF16)
            parts = [fn(part, B * (row % B) + row // B) for row in range(row0, row0 + M)]
            row = jax.lax.broadcasted_iota(jnp.int32, parts[0].shape, 0)
            merged = parts[0]
            for r in range(1, M):
                merged = jnp.where(row == r, parts[r], merged)
            halves.append(merged)
        return jnp.concatenate(halves, axis=0)

    def scores(i, slot, npages):
        return per_stream(qs[i], lambda q, s: jax.lax.dot_general(
            q, k_ring[slot, s, 0:npages].reshape(-1, DH), (((1,), (1,)), ((), ())),
            preferred_element_type=F32)) * (DH ** -0.5)

    def softmax_step(i, s):
        old = run_max[i]
        new = jnp.maximum(old, jnp.max(s, axis=-1, keepdims=True))
        p = jnp.exp(s - new[:, 0:1])
        scale = jnp.exp(old - new)
        run_max[i] = new
        run_sum[i] = scale * run_sum[i] + jnp.sum(p, axis=-1, keepdims=True)
        run_pv[i] = scale * run_pv[i]
        return p

    def accumulate(i, slot, npages, p):
        run_pv[i] += per_stream(p, lambda w, s: jnp.dot(
            w, v_ring[slot, s, 0:npages].reshape(-1, DH), preferred_element_type=F32))

    def project(i):
        heads = run_pv[i] / run_sum[i]
        total = a_acc[...]
        for c in range(H // HS):
            rows = heads[c // 2 * M:(c // 2 + 1) * M]
            if c % 2:
                rows = pltpu.roll(rows, B, 0)
            total += times_slab(rows.astype(BF16), wo, HS * c + i)
        a_acc[...] = total

    @pl.loop(0, N_A // NS)
    def _(j):
        for_streams(lambda s, fast: start_weight(
            wq_hbm, wq, w_sem.at[0], s * (N_A // NS) + j, N_A, fast))

    small = [pltpu.make_async_copy(src, dst, small_sem)
             for src, dst in ((x_hbm, x_in), (wr_hbm, wr), (gw_hbm, gw))]
    for copy in small:
        copy.start()
    start_first(k_hbm, k_ring, k_sem)
    start_first(v_hbm, v_ring, v_sem)
    for copy in small:
        copy.wait()

    xs[0:B, :] = x_in[...].astype(F32)
    xs[B:M, :] = x_in[...].astype(F32)
    y_acc[...] = jnp.zeros(y_acc.shape, F32)
    a_acc[...] = jnp.zeros(a_acc.shape, F32)
    run_max[...] = jnp.full(run_max.shape, LOWEST, F32)
    run_sum[...] = jnp.zeros(run_sum.shape, F32)
    run_pv[...] = jnp.zeros(run_pv.shape, F32)

    @pl.loop(1 - DEPTH, STEPS)
    def _(j):
        i, slot = j // JH, j % DEPTH
        first = jnp.logical_and(j >= 0, j % JH == 0)
        before = (i + HS - 1) % HS

        @pl.when(j >= 0)
        def _():
            wait_all(k_ring.at[slot], k_sem.at[slot])
            s = scores(i, slot, BLOCK)
            key = jax.lax.broadcasted_iota(jnp.int32, s.shape, 1)
            p_new[...] = softmax_step(i, jnp.where(key < jnp.where(first, OLD, 0), -jnp.inf, s))

        @pl.when(first)
        def _():
            p_old[...] = softmax_step(before, scores(before, slot, LEAD))

        @pl.when(j + DEPTH < STEPS)
        def _():
            start_cache(k_hbm, k_ring, k_sem, j + DEPTH)

        start_weight(wg_hbm, wg, w_sem.at[1], j, N_F)
        start_weight(wd_hbm, wd, w_sem.at[2], j - N_F, N_D)

        @pl.when(j + DEPTH == STEPS)
        def _():
            @pl.loop(0, TAIL * SLAB)
            def _(n):
                part = pl.ds((N_D + n) * BLOCK, BLOCK)
                start_pages(wd_hbm.at[part], wd.reshape(wd_hbm.shape).at[part],
                            tail_sem.at[n // SLAB])

        @pl.when(j >= 0)
        def _():
            wait_all(v_ring.at[slot], v_sem.at[slot])
            accumulate(i, slot, BLOCK, p_new[...])

        @pl.when(first)
        def _():
            accumulate(before, slot, LEAD, p_old[...])

        @pl.when(j + DEPTH < STEPS)
        def _():
            start_cache(v_hbm, v_ring, v_sem, j + DEPTH)

        start_weight(wu_hbm, wu, w_sem.at[3], j, N_F)
        start_weight(wo_hbm, wo, w_sem.at[4], j - N_F, N_A)

        @pl.when(j == 1 - DEPTH)
        def _():
            wait_all(wq, w_sem.at[0])

        @pl.when(j < 0)
        def _():
            share = H // 4 // (DEPTH - 1)

            @pl.loop(0, share)
            def _(n):
                c = (j + DEPTH - 1) * share + n
                for t, q in enumerate(times_tiles(xs[...].astype(BF16), wq[:, c])):
                    q_all[4 * c + t] = q

        @pl.when(j == -1)
        def _():
            upper = jax.lax.broadcasted_iota(jnp.int32, (HS, M, DH), 1) >= B
            for half in range(NS // M):
                h0 = 2 * half * HS
                qs[:, half * M:(half + 1) * M] = jnp.where(
                    upper, q_all[h0 + HS:h0 + 2 * HS], q_all[h0:h0 + HS])

        @pl.when(j == T_FFN)
        def _():
            wait_all(wg, w_sem.at[1])
            wait_all(wd.at[pl.ds(0, N_D // SLAB * 16)], w_sem.at[2])
            wait_all(wu, w_sem.at[3])

        @pl.when(between(j - T_FFN, 0, F // 512))
        def _():
            c = j - T_FFN
            x16 = xs[...].astype(BF16)
            for t, (g, u) in enumerate(zip(times_tiles(x16, wg[:, c]), times_tiles(x16, wu[:, c]))):
                act[4 * c + t] = (g * jax.nn.sigmoid(g)) * u

        @pl.when(between(j - T_FFN, 0, N_D // SLAB))
        def _():
            y_acc[...] += times_slab(act[j - T_FFN].astype(BF16), wd, j - T_FFN)

        @pl.when(j == T_OUT)
        def _():
            wait_all(wo, w_sem.at[4])

        @pl.when(jnp.logical_or(between(j - T_OUT, 0, HS - 1), j == STEPS - 1))
        def _():
            project(jnp.minimum(j - T_OUT, HS - 1))

    x = xs[...]
    gate, router = (
        jax.nn.sigmoid(jnp.sum(x * w[...].astype(F32).reshape(1, D), axis=-1, keepdims=True))
        for w in (gw, wr))

    @pl.loop(0, TAIL, init_carry=y_acc[...])
    def y(n, total):
        slab = N_D // SLAB + n
        lhs = act[slab].astype(BF16)
        wait_all(wd.at[pl.ds(slab * 16, 16)], tail_sem.at[n])
        return total + times_slab(lhs, wd, slab)

    out = gate * a_acc[...] + (1.0 - gate) * (x + (x * 0.0 + y * router))
    out_ref[...] = out[0:B, :].astype(out_ref.dtype)


def _pages(w):
    r, c = w.shape
    return w.reshape(r // 8, 8, c // 128, 128).transpose(0, 2, 1, 3).reshape(-1, PAGE, 128)


@jax.jit
def pallas_gated_mix__mha_block_cached__moe_arch_mod__decode_kernel(
    A_x: jax.Array,
    A_k_cache: jax.Array,
    A_v_cache: jax.Array,
    A_wq: jax.Array,
    A_wo: jax.Array,
    B_x: jax.Array,
    B_w_r: jax.Array,
    B_w_gate: jax.Array,
    B_w_up: jax.Array,
    B_w_down: jax.Array,
    gate_w: jax.Array,
):
    del B_x
    dma_sem = pltpu.SemaphoreType.DMA

    def resident(rows, cols):
        return pltpu.VMEM((rows // 8, cols // 512, PAGE, 128), BF16)

    out = pl.pallas_call(
        _kernel,
        out_shape=jax.ShapeDtypeStruct((B, D), BF16),
        in_specs=[pl.BlockSpec(memory_space=pl.ANY)] * 10,
        out_specs=pl.BlockSpec(memory_space=pltpu.VMEM),
        scratch_shapes=[
            pltpu.VMEM((DEPTH, NS, BLOCK, PAGE, DH), BF16),
            pltpu.VMEM((DEPTH, NS, BLOCK, PAGE, DH), BF16),
            resident(D, H * DH),
            resident(H * DH, D),
            resident(D, F),
            resident(D, F),
            resident(F, D),
            pltpu.VMEM((B, D), BF16),
            pltpu.VMEM((D,), BF16),
            pltpu.VMEM((D,), BF16),
            pltpu.VMEM((M, D), F32),
            pltpu.VMEM((H, M, DH), F32),
            pltpu.VMEM((HS, NS, DH), F32),
            pltpu.VMEM((HS, NS, 128), F32),
            pltpu.VMEM((HS, NS, 128), F32),
            pltpu.VMEM((HS, NS, DH), F32),
            pltpu.VMEM((NS, OLD), F32),
            pltpu.VMEM((NS, KEYS), F32),
            pltpu.VMEM((F // 128, M, 128), F32),
            pltpu.VMEM((M, D), F32),
            pltpu.VMEM((M, D), F32),
            dma_sem((DEPTH,)),
            dma_sem((DEPTH,)),
            dma_sem((5,)),
            dma_sem((TAIL,)),
            dma_sem,
        ],
        compiler_params=pltpu.CompilerParams(
            vmem_limit_bytes=64 * 1024 * 1024,
            disable_bounds_checks=True,
            disable_semaphore_checks=True,
        ),
    )(A_x.reshape(B, D), A_k_cache.reshape(-1, PAGE, DH), A_v_cache.reshape(-1, PAGE, DH),
      _pages(A_wq), _pages(A_wo), B_w_r, _pages(B_w_gate), _pages(B_w_up), _pages(B_w_down),
      gate_w)
    return out.reshape(B, 1, D)
```

```python
import jax
import jax.experimental.pallas as pl
import jax.experimental.pallas.tpu as pltpu
import jax.numpy as jnp
import numpy as np

B, D, H, SK, DH, F = 4, 1024, 32, 8192, 128, 3584

M = 8
PAGE = 32
BLOCK = 8
LEAD = 2
FAST = (4, 2)
NS = 16
HS = B * H // NS
KEYS = BLOCK * PAGE
OLD = LEAD * PAGE
JH = SK // KEYS
STEPS = HS * JH
DEPTH = 3
N_F = D * F // (KEYS * 128)
N_A = D * H * DH // (KEYS * 128)
SLAB = 128 * D // (KEYS * 128)
TAIL = 4
N_D = N_F - TAIL * SLAB
T_UP = N_F + DEPTH
T_DOWN = N_F + N_D + DEPTH
T_OUT = N_F + N_A + DEPTH
assert T_DOWN + N_D // SLAB < STEPS and STEPS - JH <= T_OUT and T_OUT + HS < STEPS

F32, BF16 = jnp.float32, jnp.bfloat16
LOWEST = float(np.finfo(np.float32).min)


def _kernel(x_hbm, k_hbm, v_hbm, wq_hbm, wo_hbm, wr_hbm, wg_hbm, wu_hbm, wd_hbm, gw_hbm,
            out_ref,
            k_ring, v_ring, wq, wo, wg, wu, wd, x_in, wr, gw,
            xs, gate, router, q_acc, g_acc, u_acc, y_acc, a_acc,
            qs, run_max, run_sum, run_pv, p_old, p_new,
            k_sem, v_sem, w_sem, tail_sem, small_sem):

    def between(n, lo, hi):
        return jnp.logical_and(n >= lo, n < hi)

    def wait_all(buf, sem):
        pltpu.make_async_copy(buf, buf, sem).wait()

    def start_pages(src, dst, sem, fast=FAST[0]):
        for queue, rows in enumerate((pl.ds(0, fast), pl.ds(fast, PAGE - fast))):
            pltpu.make_async_copy(src.at[:, rows], dst.at[:, rows], sem).start(priority=queue)

    def for_streams(body):
        @pl.loop(0, NS // 2)
        def _(n):
            high = ((n & 1) << 3) + (((n >> 1) & 1) << 2) + ((n >> 2) & 1)
            for low in range(2):
                body(high + 2 * low, FAST[low])

    def start_weight(src, dst, sem, n, count, fast=FAST[0]):
        @pl.when(n == 0)
        def _():
            for part in (pl.ds(count * BLOCK - LEAD, LEAD), pl.ds(0, BLOCK - LEAD)):
                start_pages(src.at[part], dst.at[part], sem, fast)

        @pl.when(between(n, 1, count))
        def _():
            part = pl.ds(n * BLOCK - LEAD, BLOCK)
            start_pages(src.at[part], dst.at[part], sem, fast)

    def start_first(src, ring, sem):
        def body(s, fast):
            prev = (s + NS - 1) % NS
            start_pages(src.at[pl.ds((prev + 1) * STEPS * BLOCK - LEAD, LEAD)],
                        ring.at[0, prev, pl.ds(0, LEAD)], sem.at[0], fast)
            start_pages(src.at[pl.ds(s * STEPS * BLOCK, BLOCK - LEAD)],
                        ring.at[0, s, pl.ds(LEAD, BLOCK - LEAD)], sem.at[0], fast)
        for_streams(body)

    def start_cache(src, ring, sem, j):
        slot = j % DEPTH
        for_streams(lambda s, fast: start_pages(
            src.at[pl.ds((s * STEPS + j) * BLOCK - LEAD, BLOCK)],
            ring.at[slot, s], sem.at[slot], fast))

    def slab(w, n, cols):
        return w.at[pl.ds(n * (cols // PAGE), cols // PAGE)]

    def times(lhs, rows):
        bands = rows[...].reshape(16, -1, PAGE, 128)
        return jnp.stack([
            jnp.dot(lhs.astype(BF16), bands[:, c, r:r + 8].reshape(128, 128),
                    preferred_element_type=F32)
            for c in range(bands.shape[1]) for r in range(0, PAGE, 8)])

    def per_stream(lhs, fn):
        halves = []
        for row0 in range(0, NS, M):
            part = lhs[row0:row0 + M].astype(BF16)
            parts = [fn(part, B * (row % B) + row // B) for row in range(row0, row0 + M)]
            row = jax.lax.broadcasted_iota(jnp.int32, parts[0].shape, 0)
            merged = parts[0]
            for r in range(1, M):
                merged = jnp.where(row == r, parts[r], merged)
            halves.append(merged)
        return jnp.concatenate(halves, axis=0)

    def scores(i, slot, npages):
        return per_stream(qs[i], lambda q, s: jax.lax.dot_general(
            q, k_ring[slot, s, 0:npages].reshape(-1, DH), (((1,), (1,)), ((), ())),
            preferred_element_type=F32)) * (DH ** -0.5)

    def softmax_step(i, s):
        old = run_max[i]
        new = jnp.maximum(old, jnp.max(s, axis=-1, keepdims=True))
        p = jnp.exp(s - new[:, 0:1])
        scale = jnp.exp(old - new)
        run_max[i] = new
        run_sum[i] = scale * run_sum[i] + jnp.sum(p, axis=-1, keepdims=True)
        run_pv[i] = scale * run_pv[i]
        return p

    def accumulate(i, slot, npages, p):
        run_pv[i] += per_stream(p, lambda w, s: jnp.dot(
            w, v_ring[slot, s, 0:npages].reshape(-1, DH), preferred_element_type=F32))

    def hidden(n):
        g = g_acc[n]
        return (g * jax.nn.sigmoid(g)) * u_acc[n]

    def project(i):
        heads = run_pv[i] / run_sum[i]
        total = a_acc[...]
        for c in range(H // HS):
            rows = heads[c // 2 * M:(c // 2 + 1) * M]
            if c % 2:
                rows = pltpu.roll(rows, B, 0)
            total += times(rows, slab(wo, HS * c + i, D))
        a_acc[...] = total

    @pl.loop(0, N_A // NS)
    def _(j):
        for_streams(lambda s, fast: start_weight(
            wq_hbm, wq, w_sem.at[0], s * (N_A // NS) + j, N_A, fast))

    small = [pltpu.make_async_copy(src, dst, small_sem)
             for src, dst in ((x_hbm, x_in), (wr_hbm, wr), (gw_hbm, gw))]
    for copy in small:
        copy.start()
    start_first(k_hbm, k_ring, k_sem)
    start_first(v_hbm, v_ring, v_sem)
    for copy in small:
        copy.wait()

    x = x_in[...].astype(F32)
    x = jnp.concatenate([x, x], axis=0)
    for n in range(D // 128):
        xs[n] = x[:, n * 128:(n + 1) * 128]
    for w, dst in ((gw, gate), (wr, router)):
        logit = jnp.sum(x * w[...].astype(F32).reshape(1, D), axis=-1, keepdims=True)
        dst[...] = jnp.broadcast_to(jax.nn.sigmoid(logit), dst.shape)
    for acc in (q_acc, g_acc, u_acc, y_acc, a_acc, run_sum, run_pv):
        acc[...] = jnp.zeros(acc.shape, F32)
    run_max[...] = jnp.full(run_max.shape, LOWEST, F32)

    @pl.loop(1 - DEPTH, STEPS)
    def _(j):
        i, slot = j // JH, j % DEPTH
        first = jnp.logical_and(j >= 0, j % JH == 0)
        before = (i + HS - 1) % HS

        @pl.when(j >= 0)
        def _():
            wait_all(k_ring.at[slot], k_sem.at[slot])
            s = scores(i, slot, BLOCK)
            key = jax.lax.broadcasted_iota(jnp.int32, s.shape, 1)
            p_new[...] = softmax_step(i, jnp.where(key < jnp.where(first, OLD, 0), -jnp.inf, s))

        @pl.when(first)
        def _():
            p_old[...] = softmax_step(before, scores(before, slot, LEAD))

        @pl.when(j + DEPTH < STEPS)
        def _():
            start_cache(k_hbm, k_ring, k_sem, j + DEPTH)

        start_weight(wg_hbm, wg, w_sem.at[1], j, N_F)
        start_weight(wd_hbm, wd, w_sem.at[2], j - N_F, N_D)

        @pl.when(j + DEPTH == STEPS)
        def _():
            @pl.loop(0, TAIL * SLAB)
            def _(n):
                part = pl.ds((N_D + n) * BLOCK, BLOCK)
                start_pages(wd_hbm.at[part], wd.at[part],
                            tail_sem.at[n // SLAB])

        @pl.when(j >= 0)
        def _():
            wait_all(v_ring.at[slot], v_sem.at[slot])
            accumulate(i, slot, BLOCK, p_new[...])

        @pl.when(first)
        def _():
            accumulate(before, slot, LEAD, p_old[...])

        @pl.when(j + DEPTH < STEPS)
        def _():
            start_cache(v_hbm, v_ring, v_sem, j + DEPTH)

        start_weight(wu_hbm, wu, w_sem.at[3], j, N_F)
        start_weight(wo_hbm, wo, w_sem.at[4], j - N_F, N_A)

        @pl.when(j == 1 - DEPTH)
        def _():
            wait_all(wq, w_sem.at[0])

        @pl.when(j < 0)
        def _():
            share = D // 128 // (DEPTH - 1)

            @pl.loop(0, share)
            def _(n):
                n += (j + DEPTH - 1) * share
                q_acc[...] += times(xs[n], slab(wq, n, H * DH))

        @pl.when(j == -1)
        def _():
            upper = jax.lax.broadcasted_iota(jnp.int32, (HS, M, DH), 1) >= B
            for half in range(NS // M):
                h0 = 2 * half * HS
                qs[:, half * M:(half + 1) * M] = jnp.where(
                    upper, q_acc[h0 + HS:h0 + 2 * HS], q_acc[h0:h0 + HS])

        @pl.when(j == T_UP)
        def _():
            wait_all(wg, w_sem.at[1])
            wait_all(wu, w_sem.at[3])

        @pl.when(between(j - T_UP, 0, D // 128))
        def _():
            n = j - T_UP
            g_acc[...] += times(xs[n], slab(wg, n, F))
            u_acc[...] += times(xs[n], slab(wu, n, F))

        @pl.when(j == T_DOWN)
        def _():
            wait_all(wd.at[pl.ds(0, N_D * BLOCK)], w_sem.at[2])

        @pl.when(between(j - T_DOWN, 0, N_D // SLAB))
        def _():
            y_acc[...] += times(hidden(j - T_DOWN), slab(wd, j - T_DOWN, D))

        @pl.when(j == T_OUT)
        def _():
            wait_all(wo, w_sem.at[4])

        @pl.when(jnp.logical_or(between(j - T_OUT, 0, HS - 1), j == STEPS - 1))
        def _():
            project(jnp.minimum(j - T_OUT, HS - 1))

    @pl.loop(0, TAIL, init_carry=y_acc[...])
    def y(n, total):
        lhs, rows = hidden(N_D // SLAB + n), slab(wd, N_D // SLAB + n, D)
        wait_all(rows, tail_sem.at[n])
        return total + times(lhs, rows)

    x, g = xs[...], gate[...]
    out = g * a_acc[...] + (1.0 - g) * (x + (x * 0.0 + y * router[...]))
    out = jnp.concatenate([out[n] for n in range(D // 128)], axis=1)
    out_ref[...] = out[0:B, :].astype(out_ref.dtype)


def _pages(w):
    r, c = w.shape
    return w.reshape(r // 8, 8, c // 128, 128).transpose(0, 2, 1, 3).reshape(-1, PAGE, 128)


@jax.jit
def pallas_gated_mix__mha_block_cached__moe_arch_mod__decode_kernel(
    A_x: jax.Array,
    A_k_cache: jax.Array,
    A_v_cache: jax.Array,
    A_wq: jax.Array,
    A_wo: jax.Array,
    B_x: jax.Array,
    B_w_r: jax.Array,
    B_w_gate: jax.Array,
    B_w_up: jax.Array,
    B_w_down: jax.Array,
    gate_w: jax.Array,
):
    del B_x
    dma_sem = pltpu.SemaphoreType.DMA

    def resident(blocks):
        return pltpu.VMEM((blocks * BLOCK, PAGE, 128), BF16)

    def tiles(cols):
        return pltpu.VMEM((cols // 128, M, 128), F32)

    out = pl.pallas_call(
        _kernel,
        out_shape=jax.ShapeDtypeStruct((B, D), BF16),
        in_specs=[pl.BlockSpec(memory_space=pl.ANY)] * 10,
        out_specs=pl.BlockSpec(memory_space=pltpu.VMEM),
        scratch_shapes=[
            pltpu.VMEM((DEPTH, NS, BLOCK, PAGE, DH), BF16),
            pltpu.VMEM((DEPTH, NS, BLOCK, PAGE, DH), BF16),
            resident(N_A),
            resident(N_A),
            resident(N_F),
            resident(N_F),
            resident(N_F),
            pltpu.VMEM((B, D), BF16),
            pltpu.VMEM((D,), BF16),
            pltpu.VMEM((D,), BF16),
            tiles(D),
            pltpu.VMEM((M, 128), F32),
            pltpu.VMEM((M, 128), F32),
            tiles(H * DH),
            tiles(F),
            tiles(F),
            tiles(D),
            tiles(D),
            pltpu.VMEM((HS, NS, DH), F32),
            pltpu.VMEM((HS, NS, 128), F32),
            pltpu.VMEM((HS, NS, 128), F32),
            pltpu.VMEM((HS, NS, DH), F32),
            pltpu.VMEM((NS, OLD), F32),
            pltpu.VMEM((NS, KEYS), F32),
            dma_sem((DEPTH,)),
            dma_sem((DEPTH,)),
            dma_sem((5,)),
            dma_sem((TAIL,)),
            dma_sem,
        ],
        compiler_params=pltpu.CompilerParams(
            vmem_limit_bytes=64 * 1024 * 1024,
            disable_bounds_checks=True,
            disable_semaphore_checks=True,
        ),
    )(A_x.reshape(B, D), A_k_cache.reshape(-1, PAGE, DH), A_v_cache.reshape(-1, PAGE, DH),
      _pages(A_wq), _pages(A_wo), B_w_r, _pages(B_w_gate), _pages(B_w_up), _pages(B_w_down),
      gate_w)
    return out.reshape(B, 1, D)
```

```python
import jax
import jax.experimental.pallas as pl
import jax.experimental.pallas.tpu as pltpu
import jax.numpy as jnp
import numpy as np

B, D, H, SK, DH, F = 4, 1024, 32, 8192, 128, 3584

M = 8
KEYS = 256
HALF = KEYS // 2
OLD = KEYS // 4
PAGE = 32
BLOCK, LEAD = KEYS // PAGE, OLD // PAGE
NS = 16
HS = B * H // NS
JH = SK // KEYS
STEPS = HS * JH
DEPTH = 2
N_F = D * F // (KEYS * 128)
N_A = D * H * DH // (KEYS * 128)
SLAB = 128 * D // (KEYS * 128)
TAIL = 4
N_D = N_F - TAIL * SLAB
assert N_F % NS == 0 and N_D % NS == 0 and N_A // NS <= D // 128 and HS < JH

F32, BF16 = jnp.float32, jnp.bfloat16
LOWEST = float(np.finfo(np.float32).min)


def _kernel(x_hbm, k_hbm, v_hbm, wq_hbm, wo_hbm, wr_hbm, wg_hbm, wu_hbm, wd_hbm, gw_hbm,
            out_ref,
            k_ring, v_ring, wq, wo, wg, wu, wd, x_in, wr, gw,
            xs, gate, router, q_acc, g_acc, u_acc, y_acc, a_acc,
            qs, run_max, run_sum, run_pv, p_old,
            k_sem, v_sem, w_sem, tail_sem, small_sem):

    def wait_all(buf, sem):
        pltpu.make_async_copy(buf, buf, sem).wait()

    def for_streams(body):
        @pl.loop(0, NS // 2)
        def _(n):
            s = ((n & 1) * 8) ^ (((n >> 1) & 1) * 2) ^ (((n >> 2) & 1) * 1)
            body(s, 0)
            body(s ^ 4, 1)

    def start_pages(src, dst, sem, pages, fast):
        for queue, rows in enumerate((pl.ds(0, fast), pl.ds(fast, PAGE - fast))):
            pltpu.make_async_copy(
                src.at[pages, rows], dst.at[pages, rows], sem).start(priority=queue)

    def start_weights(src, dst, sem, count, j):
        def body(s, odd):
            n, fast = s * (count // NS) + j, 2 if odd else 4

            @pl.when(n == 0)
            def _():
                start_pages(src, dst, sem, pl.ds(count * BLOCK - LEAD, LEAD), fast)
                start_pages(src, dst, sem, pl.ds(0, BLOCK - LEAD), fast)

            @pl.when(n > 0)
            def _():
                start_pages(src, dst, sem, pl.ds(n * BLOCK - LEAD, BLOCK), fast)

        pl.when(j < count // NS)(lambda: for_streams(body))

    def start_keys(src, dst, sem, runs):
        for queue in range(2):
            for s, row, at, count in runs:
                pltpu.make_async_copy(
                    src.at[pl.ds((s * STEPS * KEYS + row) >> 2, count // 4),
                           pl.ds(2 * queue, 2)],
                    dst.at[s, pl.ds(at % HALF // 4, count // 4),
                           pl.ds(at // HALF * 4 + 2 * queue, 2)],
                    sem).start(priority=queue)

    def start_first(src, ring, sem):
        for_streams(lambda s, _: start_keys(src, ring.at[0], sem.at[0], (
            ((s + NS - 1) % NS, STEPS * KEYS - OLD, 0, OLD),
            (s, 0, OLD, HALF - OLD),
            (s, HALF - OLD, HALF, HALF))))

    def start_cache(src, ring, sem, j):
        row, slot = j * KEYS - OLD, j % DEPTH
        for_streams(lambda s, _: start_keys(src, ring.at[slot], sem.at[slot], (
            (s, row, 0, HALF), (s, row + HALF, HALF, HALF))))

    def is_old(s):
        key = jax.lax.broadcasted_iota(jnp.int32, s.shape, 1)
        return jnp.logical_and(key < 2 * OLD, (key & 4) == 0)

    def slab(w, n, cols):
        return w.at[pl.ds(n * (cols // PAGE), cols // PAGE)]

    def times(lhs, rows):
        bands = rows[...].reshape(16, -1, PAGE, 128)
        return jnp.stack([
            jnp.dot(lhs.astype(BF16), bands[:, c, r:r + 8].reshape(128, 128),
                    preferred_element_type=F32)
            for c in range(bands.shape[1]) for r in range(0, PAGE, 8)])

    def per_stream(lhs, fn):
        halves = []
        for row0 in range(0, NS, M):
            part = lhs[row0:row0 + M].astype(BF16)
            parts = [fn(part, B * (row % B) + row // B) for row in range(row0, row0 + M)]
            row = jax.lax.broadcasted_iota(jnp.int32, parts[0].shape, 0)
            merged = parts[0]
            for r in range(1, M):
                merged = jnp.where(row == r, parts[r], merged)
            halves.append(merged)
        return jnp.concatenate(halves, axis=0)

    def scores(i, slot, keys):
        return per_stream(qs[i], lambda q, s: jax.lax.dot_general(
            q, k_ring[slot, s, 0:keys // 8].reshape(keys, DH), (((1,), (1,)), ((), ())),
            preferred_element_type=F32)) * (DH ** -0.5)

    def softmax_step(i, s):
        old = run_max[i]
        new = jnp.maximum(old, jnp.max(s, axis=-1, keepdims=True))
        p = jnp.exp(s - new[:, 0:1])
        scale = jnp.exp(old - new)
        run_max[i] = new
        run_sum[i] = scale * run_sum[i] + jnp.sum(p, axis=-1, keepdims=True)
        run_pv[i] = scale * run_pv[i]
        return p

    def accumulate(i, slot, p):
        keys = p.shape[1]
        run_pv[i] += per_stream(p, lambda w, s: jnp.dot(
            w, v_ring[slot, s, 0:keys // 8].reshape(keys, DH), preferred_element_type=F32))

    def hidden(n):
        g = g_acc[n]
        return (g * jax.nn.sigmoid(g)) * u_acc[n]

    def project(i):
        heads = run_pv[i] / run_sum[i]
        total = a_acc[...]
        for c in range(H // HS):
            rows = heads[c // 2 * M:(c // 2 + 1) * M]
            if c % 2:
                rows = pltpu.roll(rows, B, 0)
            total += times(rows, slab(wo, HS * c + i, D))
        a_acc[...] = total

    pl.loop(0, N_A // NS)(lambda j: start_weights(wq_hbm, wq, w_sem.at[0], N_A, j))
    small = [pltpu.make_async_copy(src, dst, small_sem)
             for src, dst in ((x_hbm, x_in), (wr_hbm, wr), (gw_hbm, gw))]
    for copy in small:
        copy.start()
    pl.loop(0, N_F // NS)(lambda j: start_weights(wg_hbm, wg, w_sem.at[1], N_F, j))
    for copy in small:
        copy.wait()

    x = x_in[...].astype(F32)
    x = jnp.concatenate([x, x], axis=0)
    for n in range(D // 128):
        xs[n] = x[:, n * 128:(n + 1) * 128]
    for w, dst in ((gw, gate), (wr, router)):
        logit = jnp.sum(x * w[...].astype(F32).reshape(1, D), axis=-1, keepdims=True)
        dst[...] = jnp.broadcast_to(jax.nn.sigmoid(logit), dst.shape)
    for acc in (q_acc, g_acc, u_acc, y_acc, a_acc, run_sum, run_pv):
        acc[...] = jnp.zeros(acc.shape, F32)
    run_max[...] = jnp.full(run_max.shape, LOWEST, F32)

    for n, (w, acc, arriving) in enumerate((
            (wq, q_acc, (wu_hbm, wu, w_sem.at[2], N_F)),
            (wg, g_acc, (wo_hbm, wo, w_sem.at[3], N_A)),
            (wu, u_acc, (wd_hbm, wd, w_sem.at[4], N_D)))):
        wait_all(w, w_sem.at[n])

        @pl.loop(0, D // 128)
        def _(j):
            start_weights(*arriving, j)
            acc[...] += times(xs[j], slab(w, j, acc.shape[0] * 128))

    upper = jax.lax.broadcasted_iota(jnp.int32, (HS, M, DH), 1) >= B
    for half in range(NS // M):
        h0 = 2 * half * HS
        qs[:, half * M:(half + 1) * M] = jnp.where(
            upper, q_acc[h0 + HS:h0 + 2 * HS], q_acc[h0:h0 + HS])

    start_first(k_hbm, k_ring, k_sem)
    start_first(v_hbm, v_ring, v_sem)
    for j in range(1, DEPTH):
        start_cache(k_hbm, k_ring, k_sem, j)
        start_cache(v_hbm, v_ring, v_sem, j)
    wait_all(wo, w_sem.at[3])
    wait_all(wd.at[pl.ds(0, N_D * BLOCK)], w_sem.at[4])

    @pl.loop(0, STEPS)
    def _(j):
        i, slot, first = j // JH, j % DEPTH, j % JH == 0
        before = (i + HS - 1) % HS

        wait_all(k_ring.at[slot], k_sem.at[slot])
        s = scores(i, slot, KEYS)
        p = softmax_step(i, jnp.where(jnp.logical_and(first, is_old(s)), -jnp.inf, s))

        @pl.when(first)
        def _():
            s = scores(before, slot, 2 * OLD)
            p_old[...] = softmax_step(before, jnp.where(is_old(s), s, -jnp.inf))

        @pl.when(j + DEPTH < STEPS)
        def _():
            start_cache(k_hbm, k_ring, k_sem, j + DEPTH)

        @pl.when(j + DEPTH == STEPS)
        def _():
            @pl.loop(0, TAIL * SLAB)
            def _(n):
                start_pages(wd_hbm, wd, tail_sem.at[n // SLAB],
                            pl.ds((N_D + n) * BLOCK, BLOCK), 4)

        wait_all(v_ring.at[slot], v_sem.at[slot])
        accumulate(i, slot, p)

        @pl.when(first)
        def _():
            accumulate(before, slot, p_old[...])

        @pl.when(j + DEPTH < STEPS)
        def _():
            start_cache(v_hbm, v_ring, v_sem, j + DEPTH)

        @pl.when(j < N_D // SLAB)
        def _():
            y_acc[...] += times(hidden(j), slab(wd, j, D))

        last = j == STEPS - 1

        @pl.when(jnp.logical_or(jnp.logical_and(first, j > 0), last))
        def _():
            project(jnp.where(last, i, before))

    @pl.loop(0, TAIL, init_carry=y_acc[...])
    def y(n, total):
        lhs, rows = hidden(N_D // SLAB + n), slab(wd, N_D // SLAB + n, D)
        wait_all(rows, tail_sem.at[n])
        return total + times(lhs, rows)

    x, g = xs[...], gate[...]
    out = g * a_acc[...] + (1.0 - g) * (x + (x * 0.0 + y * router[...]))
    out = jnp.concatenate([out[n] for n in range(D // 128)], axis=1)
    out_ref[...] = out[0:B, :].astype(out_ref.dtype)


def _pages(w):
    r, c = w.shape
    return w.reshape(r // 8, 8, c // 128, 128).transpose(0, 2, 1, 3).reshape(-1, PAGE, 128)


@jax.jit
def pallas_gated_mix__mha_block_cached__moe_arch_mod__decode_kernel(
    A_x: jax.Array,
    A_k_cache: jax.Array,
    A_v_cache: jax.Array,
    A_wq: jax.Array,
    A_wo: jax.Array,
    B_x: jax.Array,
    B_w_r: jax.Array,
    B_w_gate: jax.Array,
    B_w_up: jax.Array,
    B_w_down: jax.Array,
    gate_w: jax.Array,
):
    del B_x
    dma_sem = pltpu.SemaphoreType.DMA

    def resident(blocks):
        return pltpu.VMEM((blocks * BLOCK, PAGE, 128), BF16)

    def tiles(cols):
        return pltpu.VMEM((cols // 128, M, 128), F32)

    out = pl.pallas_call(
        _kernel,
        out_shape=jax.ShapeDtypeStruct((B, D), BF16),
        in_specs=[pl.BlockSpec(memory_space=pl.ANY)] * 10,
        out_specs=pl.BlockSpec(memory_space=pltpu.VMEM),
        scratch_shapes=[
            pltpu.VMEM((DEPTH, NS, KEYS // 8, 8, DH), BF16),
            pltpu.VMEM((DEPTH, NS, KEYS // 8, 8, DH), BF16),
            resident(N_A),
            resident(N_A),
            resident(N_F),
            resident(N_F),
            resident(N_F),
            pltpu.VMEM((B, D), BF16),
            pltpu.VMEM((D,), BF16),
            pltpu.VMEM((D,), BF16),
            tiles(D),
            pltpu.VMEM((M, 128), F32),
            pltpu.VMEM((M, 128), F32),
            tiles(H * DH),
            tiles(F),
            tiles(F),
            tiles(D),
            tiles(D),
            pltpu.VMEM((HS, NS, DH), F32),
            pltpu.VMEM((HS, NS, 128), F32),
            pltpu.VMEM((HS, NS, 128), F32),
            pltpu.VMEM((HS, NS, DH), F32),
            pltpu.VMEM((NS, 2 * OLD), F32),
            dma_sem((DEPTH,)),
            dma_sem((DEPTH,)),
            dma_sem((5,)),
            dma_sem((TAIL,)),
            dma_sem,
        ],
        compiler_params=pltpu.CompilerParams(
            vmem_limit_bytes=64 * 1024 * 1024,
            disable_bounds_checks=True,
            disable_semaphore_checks=True,
        ),
    )(A_x.reshape(B, D), A_k_cache.reshape(-1, 4, DH), A_v_cache.reshape(-1, 4, DH),
      _pages(A_wq), _pages(A_wo), B_w_r, _pages(B_w_gate), _pages(B_w_up), _pages(B_w_down),
      gate_w)
    return out.reshape(B, 1, D)
```

```python
import jax
import jax.experimental.pallas as pl
import jax.experimental.pallas.tpu as pltpu
import jax.numpy as jnp
import numpy as np

B, D, H, SK, DH, F = 4, 1024, 32, 8192, 128, 3584

M = 8
KEYS = 256
HALF = KEYS // 2
OLD = KEYS // 4
PAGE = 32
BLOCK, LEAD = KEYS // PAGE, OLD // PAGE
NS = 16
HS = B * H // NS
JH = SK // KEYS
STEPS = HS * JH
DEPTH = 2
N_F = D * F // (KEYS * 128)
N_A = D * H * DH // (KEYS * 128)
SLAB = 128 * D // (KEYS * 128)
TAIL = 4
N_D = N_F - TAIL * SLAB
assert N_F % NS == 0 and N_D % NS == 0 and N_A // NS <= D // 128

F32, BF16 = jnp.float32, jnp.bfloat16
LOWEST = float(np.finfo(np.float32).min)


def _kernel(x_hbm, k_hbm, v_hbm, wq_hbm, wo_hbm, wr_hbm, wg_hbm, wu_hbm, wd_hbm, gw_hbm,
            out_ref,
            k_ring, v_ring, wq, wo, wg, wu, wd, x_in, wr, gw,
            xs, gate, router, q_acc, g_acc, u_acc, y_acc, a_acc,
            qs, run_max, run_sum, run_pv, p_old,
            k_sem, v_sem, w_sem, tail_sem, small_sem):

    def wait_all(buf, sem):
        pltpu.make_async_copy(buf, buf, sem).wait()

    def for_streams(body):
        @pl.loop(0, NS // 4)
        def _(n):
            for high in (0, 12, 8, 4):
                body((n & 1) * 2 + (n >> 1) + high)

    def start_pages(src, dst, sem, pages, fast):
        for queue, rows in enumerate((pl.ds(0, fast), pl.ds(fast, PAGE - fast))):
            pltpu.make_async_copy(
                src.at[pages, rows], dst.at[pages, rows], sem).start(priority=queue)

    def start_weights(src, dst, sem, count, j):
        @pl.when(j < count // NS)
        def _():
            @pl.loop(0, NS // 2)
            def _(s):
                n = s * (count // NS) + j

                @pl.when(n == 0)
                def _():
                    start_pages(src, dst, sem, pl.ds(count * BLOCK - LEAD, LEAD), 4)
                    start_pages(src, dst, sem, pl.ds(0, BLOCK - LEAD), 4)

                @pl.when(n > 0)
                def _():
                    start_pages(src, dst, sem, pl.ds(n * BLOCK - LEAD, BLOCK), 4)

                start_pages(src, dst, sem, pl.ds((n + count // 2) * BLOCK - LEAD, BLOCK), 2)

    def start_keys(src, dst, sem, runs):
        for queue in range(2):
            for s, j, row, count in runs:
                pltpu.make_async_copy(
                    src.at[pl.ds((s * STEPS + j) * (KEYS // 4) + (row - OLD) // 4, count // 4),
                           pl.ds(2 * queue, 2)],
                    dst.at[s, pl.ds(row % HALF // 4, count // 4),
                           pl.ds(row // HALF * 4 + 2 * queue, 2)],
                    sem).start(priority=queue)

    def start_first(src, ring, sem):
        for_streams(lambda s: start_keys(src, ring.at[0], sem.at[0], (
            ((s + NS - 1) % NS, STEPS, 0, OLD), (s, 0, OLD, HALF - OLD), (s, 0, HALF, HALF))))

    def start_cache(src, ring, sem, j):
        slot = j % DEPTH
        for_streams(lambda s: start_keys(src, ring.at[slot], sem.at[slot], (
            (s, j, 0, HALF), (s, j, HALF, HALF))))

    def is_old(s):
        key = jax.lax.broadcasted_iota(jnp.int32, s.shape, 1)
        return jnp.logical_and(key < 2 * OLD, (key & 4) == 0)

    def slab(w, n, cols):
        return w.at[pl.ds(n * (cols // PAGE), cols // PAGE)]

    def times(lhs, rows):
        bands = rows[...].reshape(16, -1, PAGE, 128)
        return jnp.stack([
            jnp.dot(lhs.astype(BF16), bands[:, c, r:r + 8].reshape(128, 128),
                    preferred_element_type=F32)
            for c in range(bands.shape[1]) for r in range(0, PAGE, 8)])

    def per_stream(lhs, fn):
        halves = []
        for row0 in range(0, NS, M):
            part = lhs[row0:row0 + M].astype(BF16)
            parts = [fn(part, B * (row % B) + row // B) for row in range(row0, row0 + M)]
            row = jax.lax.broadcasted_iota(jnp.int32, parts[0].shape, 0)
            merged = parts[0]
            for r in range(1, M):
                merged = jnp.where(row == r, parts[r], merged)
            halves.append(merged)
        return jnp.concatenate(halves, axis=0)

    def scores(i, slot, keys):
        return per_stream(qs[i], lambda q, s: jax.lax.dot_general(
            q, k_ring[slot, s, 0:keys // 8].reshape(keys, DH), (((1,), (1,)), ((), ())),
            preferred_element_type=F32)) * (DH ** -0.5)

    def softmax_step(i, s):
        old = run_max[i]
        new = jnp.maximum(old, jnp.max(s, axis=-1, keepdims=True))
        p = jnp.exp(s - new[:, 0:1])
        scale = jnp.exp(old - new)
        run_max[i] = new
        run_sum[i] = scale * run_sum[i] + jnp.sum(p, axis=-1, keepdims=True)
        run_pv[i] = scale * run_pv[i]
        return p

    def accumulate(i, slot, p):
        keys = p.shape[1]
        run_pv[i] += per_stream(p, lambda w, s: jnp.dot(
            w, v_ring[slot, s, 0:keys // 8].reshape(keys, DH), preferred_element_type=F32))

    def hidden(n):
        g = g_acc[n]
        return (g * jax.nn.sigmoid(g)) * u_acc[n]

    def project(i):
        heads = run_pv[i] / run_sum[i]
        total = a_acc[...]
        for c in range(H // HS):
            rows = heads[c // 2 * M:(c // 2 + 1) * M]
            if c % 2:
                rows = pltpu.roll(rows, B, 0)
            total += times(rows, slab(wo, HS * c + i, D))
        a_acc[...] = total

    pl.loop(0, N_A // NS)(lambda j: start_weights(wq_hbm, wq, w_sem.at[0], N_A, j))
    small = [pltpu.make_async_copy(src, dst, small_sem)
             for src, dst in ((x_hbm, x_in), (wr_hbm, wr), (gw_hbm, gw))]
    for copy in small:
        copy.start()
    pl.loop(0, N_F // NS)(lambda j: start_weights(wg_hbm, wg, w_sem.at[1], N_F, j))
    for copy in small:
        copy.wait()

    x = x_in[...].astype(F32)
    x = jnp.concatenate([x, x], axis=0)
    for n in range(D // 128):
        xs[n] = x[:, n * 128:(n + 1) * 128]
    for w, dst in ((gw, gate), (wr, router)):
        logit = jnp.sum(x * w[...].astype(F32).reshape(1, D), axis=-1, keepdims=True)
        dst[...] = jnp.broadcast_to(jax.nn.sigmoid(logit), dst.shape)
    for acc in (q_acc, g_acc, u_acc, y_acc, a_acc, run_sum, run_pv):
        acc[...] = jnp.zeros(acc.shape, F32)
    run_max[...] = jnp.full(run_max.shape, LOWEST, F32)

    for n, (w, acc, arriving) in enumerate((
            (wq, q_acc, (wu_hbm, wu, w_sem.at[2], N_F)),
            (wg, g_acc, (wo_hbm, wo, w_sem.at[3], N_A)),
            (wu, u_acc, (wd_hbm, wd, w_sem.at[4], N_D)))):
        wait_all(w, w_sem.at[n])

        @pl.loop(0, D // 128)
        def _(j):
            start_weights(*arriving, j)
            acc[...] += times(xs[j], slab(w, j, acc.shape[0] * 128))

    upper = jax.lax.broadcasted_iota(jnp.int32, (HS, M, DH), 1) >= B
    for half in range(NS // M):
        h0 = 2 * half * HS
        qs[:, half * M:(half + 1) * M] = jnp.where(
            upper, q_acc[h0 + HS:h0 + 2 * HS], q_acc[h0:h0 + HS])

    start_first(k_hbm, k_ring, k_sem)
    start_first(v_hbm, v_ring, v_sem)
    for j in range(1, DEPTH):
        start_cache(k_hbm, k_ring, k_sem, j)
        start_cache(v_hbm, v_ring, v_sem, j)
    wait_all(wo, w_sem.at[3])
    wait_all(wd.at[pl.ds(0, N_D * BLOCK)], w_sem.at[4])

    @pl.loop(0, STEPS)
    def _(j):
        i, slot, first = j // JH, j % DEPTH, j % JH == 0
        before = (i + HS - 1) % HS

        wait_all(k_ring.at[slot], k_sem.at[slot])
        s = scores(i, slot, KEYS)
        p = softmax_step(i, jnp.where(jnp.logical_and(first, is_old(s)), -jnp.inf, s))

        @pl.when(first)
        def _():
            s = scores(before, slot, 2 * OLD)
            p_old[...] = softmax_step(before, jnp.where(is_old(s), s, -jnp.inf))

        @pl.when(j + DEPTH < STEPS)
        def _():
            start_cache(k_hbm, k_ring, k_sem, j + DEPTH)

        @pl.when(j + DEPTH == STEPS)
        def _():
            @pl.loop(0, TAIL * SLAB)
            def _(n):
                start_pages(wd_hbm, wd, tail_sem.at[n // SLAB],
                            pl.ds((N_D + n) * BLOCK, BLOCK), 4)

        wait_all(v_ring.at[slot], v_sem.at[slot])
        accumulate(i, slot, p)

        @pl.when(first)
        def _():
            accumulate(before, slot, p_old[...])

        @pl.when(j + DEPTH < STEPS)
        def _():
            start_cache(v_hbm, v_ring, v_sem, j + DEPTH)

        @pl.when(j < N_D // SLAB)
        def _():
            y_acc[...] += times(hidden(j), slab(wd, j, D))

        last = j == STEPS - 1

        @pl.when(jnp.logical_or(jnp.logical_and(first, j > 0), last))
        def _():
            project(jnp.where(last, i, before))

    @pl.loop(0, TAIL, init_carry=y_acc[...])
    def y(n, total):
        lhs, rows = hidden(N_D // SLAB + n), slab(wd, N_D // SLAB + n, D)
        wait_all(rows, tail_sem.at[n])
        return total + times(lhs, rows)

    x, g = xs[...], gate[...]
    out = g * a_acc[...] + (1.0 - g) * (x + (x * 0.0 + y * router[...]))
    out = jnp.concatenate([out[n] for n in range(D // 128)], axis=1)
    out_ref[...] = out[0:B, :].astype(out_ref.dtype)


def _pages(w):
    r, c = w.shape
    return w.reshape(r // 8, 8, c // 128, 128).transpose(0, 2, 1, 3).reshape(-1, PAGE, 128)


@jax.jit
def pallas_gated_mix__mha_block_cached__moe_arch_mod__decode_kernel(
    A_x: jax.Array,
    A_k_cache: jax.Array,
    A_v_cache: jax.Array,
    A_wq: jax.Array,
    A_wo: jax.Array,
    B_x: jax.Array,
    B_w_r: jax.Array,
    B_w_gate: jax.Array,
    B_w_up: jax.Array,
    B_w_down: jax.Array,
    gate_w: jax.Array,
):
    del B_x
    dma_sem = pltpu.SemaphoreType.DMA

    def resident(blocks):
        return pltpu.VMEM((blocks * BLOCK, PAGE, 128), BF16)

    def tiles(cols):
        return pltpu.VMEM((cols // 128, M, 128), F32)

    out = pl.pallas_call(
        _kernel,
        out_shape=jax.ShapeDtypeStruct((B, D), BF16),
        in_specs=[pl.BlockSpec(memory_space=pl.ANY)] * 10,
        out_specs=pl.BlockSpec(memory_space=pltpu.VMEM),
        scratch_shapes=[
            pltpu.VMEM((DEPTH, NS, KEYS // 8, 8, DH), BF16),
            pltpu.VMEM((DEPTH, NS, KEYS // 8, 8, DH), BF16),
            resident(N_A),
            resident(N_A),
            resident(N_F),
            resident(N_F),
            resident(N_F),
            pltpu.VMEM((B, D), BF16),
            pltpu.VMEM((D,), BF16),
            pltpu.VMEM((D,), BF16),
            tiles(D),
            pltpu.VMEM((M, 128), F32),
            pltpu.VMEM((M, 128), F32),
            tiles(H * DH),
            tiles(F),
            tiles(F),
            tiles(D),
            tiles(D),
            pltpu.VMEM((HS, NS, DH), F32),
            pltpu.VMEM((HS, NS, 128), F32),
            pltpu.VMEM((HS, NS, 128), F32),
            pltpu.VMEM((HS, NS, DH), F32),
            pltpu.VMEM((NS, 2 * OLD), F32),
            dma_sem((DEPTH,)),
            dma_sem((DEPTH,)),
            dma_sem((5,)),
            dma_sem((TAIL,)),
            dma_sem,
        ],
        compiler_params=pltpu.CompilerParams(
            vmem_limit_bytes=64 * 1024 * 1024,
            disable_bounds_checks=True,
            disable_semaphore_checks=True,
        ),
    )(A_x.reshape(B, D), A_k_cache.reshape(-1, 4, DH), A_v_cache.reshape(-1, 4, DH),
      _pages(A_wq), _pages(A_wo), B_w_r, _pages(B_w_gate), _pages(B_w_up), _pages(B_w_down),
      gate_w)
    return out.reshape(B, 1, D)
```

```python
import jax
import jax.experimental.pallas as pl
import jax.experimental.pallas.tpu as pltpu
import jax.numpy as jnp
import numpy as np

B, D, H, SK, DH, F = 4, 1024, 32, 8192, 128, 3584

M = 8
KEYS = 256
OLD = KEYS // 4
PAGE = 32
BLOCK, LEAD = KEYS // PAGE, OLD // PAGE
NS = 16
HS = B * H // NS
JH = SK // KEYS
STEPS = HS * JH
DEPTH = 2
N_F = D * F // (KEYS * 128)
N_A = D * H * DH // (KEYS * 128)
SLAB = 128 * D // (KEYS * 128)
TAIL = 4
N_D = N_F - TAIL * SLAB
assert N_F % NS == 0 and N_D % NS == 0 and N_A // NS <= D // 128

F32, BF16 = jnp.float32, jnp.bfloat16
LOWEST = float(np.finfo(np.float32).min)


def _kernel(x_hbm, k_hbm, v_hbm, wq_hbm, wo_hbm, wr_hbm, wg_hbm, wu_hbm, wd_hbm, gw_hbm,
            out_ref,
            k_ring, v_ring, wq, wo, wg, wu, wd, x_in, wr, gw,
            xs, gate, router, q_acc, g_acc, u_acc, y_acc, a_acc,
            qs, run_max, run_sum, run_pv, p_old,
            k_sem, v_sem, w_sem, tail_sem, small_sem):

    def wait_all(buf, sem):
        pltpu.make_async_copy(buf, buf, sem).wait()

    def start_pages(src, dst, sem, pages, fast):
        for queue, rows in enumerate((pl.ds(0, fast), pl.ds(fast, PAGE - fast))):
            pltpu.make_async_copy(
                src.at[pages, rows], dst.at[pages, rows], sem).start(priority=queue)

    def start_weights(src, dst, sem, count, j):
        @pl.when(j < count // NS)
        def _():
            @pl.loop(0, NS // 2)
            def _(s):
                n = s * (count // NS) + j

                @pl.when(n == 0)
                def _():
                    start_pages(src, dst, sem, pl.ds(count * BLOCK - LEAD, LEAD), 4)
                    start_pages(src, dst, sem, pl.ds(0, BLOCK - LEAD), 4)

                @pl.when(n > 0)
                def _():
                    start_pages(src, dst, sem, pl.ds(n * BLOCK - LEAD, BLOCK), 4)

                start_pages(src, dst, sem, pl.ds((n + count // 2) * BLOCK - LEAD, BLOCK), 2)

    def start_keys(src, ring, sem, slot, runs):
        for odd in range(2):
            @pl.loop(0, 2)
            def _(n):
                for p in (n, n + 6, n + 4, n + 2):
                    for queue in range(2):
                        for j, row, count in runs:
                            at = ((2 * p + odd) * STEPS + j) * (KEYS // 4) + (row - OLD) // 4
                            pltpu.make_async_copy(
                                src.at[pl.ds(at, count // 4), pl.ds(2 * queue, 2)],
                                ring.at[slot, p, pl.ds(row // 4, count // 4),
                                        pl.ds(4 * odd + 2 * queue, 2)],
                                sem.at[slot]).start(priority=queue)

    def start_first(src, ring, sem):
        start_keys(src, ring, sem, 0, ((STEPS, 0, OLD), (0, OLD, KEYS - OLD)))

    def start_cache(src, ring, sem, j):
        start_keys(src, ring, sem, j % DEPTH, ((j, 0, KEYS),))

    def slab(w, n, cols):
        return w.at[pl.ds(n * (cols // PAGE), cols // PAGE)]

    def times(lhs, rows):
        bands = rows[...].reshape(16, -1, PAGE, 128)
        return jnp.stack([
            jnp.dot(lhs.astype(BF16), bands[:, c, r:r + 8].reshape(128, 128),
                    preferred_element_type=F32)
            for c in range(bands.shape[1]) for r in range(0, PAGE, 8)])

    def per_entry(lhs, fn):
        halves = []
        for half in range(NS // M):
            part = lhs[half * M:(half + 1) * M].astype(BF16)
            parts = [fn(part, 2 * b + half) for b in range(B)]
            batch = jax.lax.broadcasted_iota(jnp.int32, parts[0].shape, 0) % B
            merged = parts[0]
            for b in range(1, B):
                merged = jnp.where(batch == b, parts[b], merged)
            halves.append(merged)
        return jnp.concatenate(halves, axis=0)

    def scores(i, slot, lo, hi):
        s = per_entry(qs[i], lambda q, p: jax.lax.dot_general(
            q, k_ring[slot, p, 0:hi // 4].reshape(2 * hi, DH), (((1,), (1,)), ((), ())),
            preferred_element_type=F32)) * (DH ** -0.5)
        row, key = (jax.lax.broadcasted_iota(jnp.int32, s.shape, d) for d in range(2))
        return jnp.where(jnp.logical_and(((row ^ key) & 4) == 0, key >= 2 * lo), s, -jnp.inf)

    def softmax_step(i, s):
        old = run_max[i]
        new = jnp.maximum(old, jnp.max(s, axis=-1, keepdims=True))
        p = jnp.exp(s - new[:, 0:1])
        scale = jnp.exp(old - new)
        run_max[i] = new
        run_sum[i] = scale * run_sum[i] + jnp.sum(p, axis=-1, keepdims=True)
        run_pv[i] = scale * run_pv[i]
        return p

    def accumulate(i, slot, p):
        keys = p.shape[1]
        run_pv[i] += per_entry(p, lambda w, e: jnp.dot(
            w, v_ring[slot, e, 0:keys // 8].reshape(keys, DH), preferred_element_type=F32))

    def hidden(n):
        g = g_acc[n]
        return (g * jax.nn.sigmoid(g)) * u_acc[n]

    def project(i):
        heads = run_pv[i] / run_sum[i]
        total = a_acc[...]
        for c in range(H // HS):
            rows = heads[c // 2 * M:(c // 2 + 1) * M]
            if c % 2:
                rows = pltpu.roll(rows, B, 0)
            total += times(rows, slab(wo, HS * c + i, D))
        a_acc[...] = total

    pl.loop(0, N_A // NS)(lambda j: start_weights(wq_hbm, wq, w_sem.at[0], N_A, j))
    small = [pltpu.make_async_copy(src, dst, small_sem)
             for src, dst in ((x_hbm, x_in), (wr_hbm, wr), (gw_hbm, gw))]
    for copy in small:
        copy.start()
    pl.loop(0, N_F // NS)(lambda j: start_weights(wg_hbm, wg, w_sem.at[1], N_F, j))
    for copy in small:
        copy.wait()

    x = x_in[...].astype(F32)
    x = jnp.concatenate([x, x], axis=0)
    for n in range(D // 128):
        xs[n] = x[:, n * 128:(n + 1) * 128]
    for w, dst in ((gw, gate), (wr, router)):
        logit = jnp.sum(x * w[...].astype(F32).reshape(1, D), axis=-1, keepdims=True)
        dst[...] = jnp.broadcast_to(jax.nn.sigmoid(logit), dst.shape)
    for acc in (q_acc, g_acc, u_acc, y_acc, a_acc, run_sum, run_pv):
        acc[...] = jnp.zeros(acc.shape, F32)
    run_max[...] = jnp.full(run_max.shape, LOWEST, F32)

    for n, (w, acc, arriving) in enumerate((
            (wq, q_acc, (wu_hbm, wu, w_sem.at[2], N_F)),
            (wg, g_acc, (wo_hbm, wo, w_sem.at[3], N_A)),
            (wu, u_acc, (wd_hbm, wd, w_sem.at[4], N_D)))):
        wait_all(w, w_sem.at[n])

        @pl.loop(0, D // 128)
        def _(j):
            start_weights(*arriving, j)
            acc[...] += times(xs[j], slab(w, j, acc.shape[0] * 128))

    upper = jax.lax.broadcasted_iota(jnp.int32, (HS, M, DH), 1) >= B
    for half in range(NS // M):
        h0 = 2 * half * HS
        qs[:, half * M:(half + 1) * M] = jnp.where(
            upper, q_acc[h0 + HS:h0 + 2 * HS], q_acc[h0:h0 + HS])

    start_first(k_hbm, k_ring, k_sem)
    start_first(v_hbm, v_ring, v_sem)
    for j in range(1, DEPTH):
        start_cache(k_hbm, k_ring, k_sem, j)
        start_cache(v_hbm, v_ring, v_sem, j)
    wait_all(wo, w_sem.at[3])
    wait_all(wd.at[pl.ds(0, N_D * BLOCK)], w_sem.at[4])

    @pl.loop(0, STEPS)
    def _(j):
        i, slot, first = j // JH, j % DEPTH, j % JH == 0
        before = (i + HS - 1) % HS

        wait_all(k_ring.at[slot], k_sem.at[slot])
        p = softmax_step(i, scores(i, slot, jnp.where(first, OLD, 0), KEYS))

        @pl.when(first)
        def _():
            p_old[...] = softmax_step(before, scores(before, slot, 0, OLD))

        @pl.when(j + DEPTH < STEPS)
        def _():
            start_cache(k_hbm, k_ring, k_sem, j + DEPTH)

        @pl.when(j + DEPTH == STEPS)
        def _():
            @pl.loop(0, TAIL * SLAB)
            def _(n):
                start_pages(wd_hbm, wd, tail_sem.at[n // SLAB],
                            pl.ds((N_D + n) * BLOCK, BLOCK), 4)

        wait_all(v_ring.at[slot], v_sem.at[slot])
        accumulate(i, slot, p)

        @pl.when(first)
        def _():
            accumulate(before, slot, p_old[...])

        @pl.when(j + DEPTH < STEPS)
        def _():
            start_cache(v_hbm, v_ring, v_sem, j + DEPTH)

        @pl.when(j < N_D // SLAB)
        def _():
            y_acc[...] += times(hidden(j), slab(wd, j, D))

        last = j == STEPS - 1

        @pl.when(jnp.logical_or(jnp.logical_and(first, j > 0), last))
        def _():
            project(jnp.where(last, i, before))

    @pl.loop(0, TAIL, init_carry=y_acc[...])
    def y(n, total):
        lhs, rows = hidden(N_D // SLAB + n), slab(wd, N_D // SLAB + n, D)
        wait_all(rows, tail_sem.at[n])
        return total + times(lhs, rows)

    x, g = xs[...], gate[...]
    out = g * a_acc[...] + (1.0 - g) * (x + (x * 0.0 + y * router[...]))
    out = jnp.concatenate([out[n] for n in range(D // 128)], axis=1)
    out_ref[...] = out[0:B, :].astype(out_ref.dtype)


def _pages(w):
    r, c = w.shape
    return w.reshape(r // 8, 8, c // 128, 128).transpose(0, 2, 1, 3).reshape(-1, PAGE, 128)


@jax.jit
def pallas_gated_mix__mha_block_cached__moe_arch_mod__decode_kernel(
    A_x: jax.Array,
    A_k_cache: jax.Array,
    A_v_cache: jax.Array,
    A_wq: jax.Array,
    A_wo: jax.Array,
    B_x: jax.Array,
    B_w_r: jax.Array,
    B_w_gate: jax.Array,
    B_w_up: jax.Array,
    B_w_down: jax.Array,
    gate_w: jax.Array,
):
    del B_x
    dma_sem = pltpu.SemaphoreType.DMA

    def resident(blocks):
        return pltpu.VMEM((blocks * BLOCK, PAGE, 128), BF16)

    def tiles(cols):
        return pltpu.VMEM((cols // 128, M, 128), F32)

    out = pl.pallas_call(
        _kernel,
        out_shape=jax.ShapeDtypeStruct((B, D), BF16),
        in_specs=[pl.BlockSpec(memory_space=pl.ANY)] * 10,
        out_specs=pl.BlockSpec(memory_space=pltpu.VMEM),
        scratch_shapes=[
            pltpu.VMEM((DEPTH, NS // 2, KEYS // 4, 8, DH), BF16),
            pltpu.VMEM((DEPTH, NS // 2, KEYS // 4, 8, DH), BF16),
            resident(N_A),
            resident(N_A),
            resident(N_F),
            resident(N_F),
            resident(N_F),
            pltpu.VMEM((B, D), BF16),
            pltpu.VMEM((D,), BF16),
            pltpu.VMEM((D,), BF16),
            tiles(D),
            pltpu.VMEM((M, 128), F32),
            pltpu.VMEM((M, 128), F32),
            tiles(H * DH),
            tiles(F),
            tiles(F),
            tiles(D),
            tiles(D),
            pltpu.VMEM((HS, NS, DH), F32),
            pltpu.VMEM((HS, NS, 128), F32),
            pltpu.VMEM((HS, NS, 128), F32),
            pltpu.VMEM((HS, NS, DH), F32),
            pltpu.VMEM((NS, 2 * OLD), F32),
            dma_sem((DEPTH,)),
            dma_sem((DEPTH,)),
            dma_sem((5,)),
            dma_sem((TAIL,)),
            dma_sem,
        ],
        compiler_params=pltpu.CompilerParams(
            vmem_limit_bytes=64 * 1024 * 1024,
            disable_bounds_checks=True,
            disable_semaphore_checks=True,
        ),
    )(A_x.reshape(B, D), A_k_cache.reshape(-1, 4, DH), A_v_cache.reshape(-1, 4, DH),
      _pages(A_wq), _pages(A_wo), B_w_r, _pages(B_w_gate), _pages(B_w_up), _pages(B_w_down),
      gate_w)
    return out.reshape(B, 1, D)
```

```python
import jax
import jax.experimental.pallas as pl
import jax.experimental.pallas.tpu as pltpu
import jax.numpy as jnp
import numpy as np

B, D, H, SK, DH, F = 4, 1024, 32, 8192, 128, 3584

M = 8
KEYS = 256
OLD = KEYS // 4
PAGE = 32
BLOCK, LEAD = KEYS // PAGE, OLD // PAGE
NS = 16
HS = B * H // NS
JH = SK // KEYS
STEPS = HS * JH
DEPTH = 2
N_F = D * F // (KEYS * 128)
N_A = D * H * DH // (KEYS * 128)
SLAB = 128 * D // (KEYS * 128)
TAIL = 4
N_D = N_F - TAIL * SLAB
assert N_F % NS == 0 and N_D % NS == 0 and N_A // NS <= D // 128 and N_D // SLAB < STEPS

K_ORDER = (0, 8, 25, 17, 21, 29, 12, 4, 10, 2, 26, 7, 19, 23, 31, 14)
V_ORDER = (2, 6, 14, 12, 29, 21, 19, 27, 10, 4, 0, 16, 24, 9, 22, 30)
assert all(sorted(n // 2 for n in order) == list(range(NS)) for order in (K_ORDER, V_ORDER))

F32, BF16 = jnp.float32, jnp.bfloat16
LOWEST = float(np.finfo(np.float32).min)


def _kernel(x_hbm, k_hbm, v_hbm, wq_hbm, wo_hbm, wr_hbm, wg_hbm, wu_hbm, wd_hbm, gw_hbm,
            out_ref,
            k_ring, v_ring, wq, wo, wg, wu, wd, x_in, wr, gw,
            xs, gate, router, q_acc, g_acc, u_acc, y_acc, a_acc,
            qs, run_max, run_sum, run_pv, p_old,
            k_sem, v_sem, w_sem, tail_sem, small_sem):

    def wait_all(buf, sem):
        pltpu.make_async_copy(buf, buf, sem).wait()

    def start_pages(src, dst, sem, pages, fast):
        for queue, rows in enumerate((pl.ds(0, fast), pl.ds(fast, PAGE - fast))):
            pltpu.make_async_copy(
                src.at[pages, rows], dst.at[pages, rows], sem).start(priority=queue)

    def start_weights(src, dst, sem, count, j):
        @pl.when(j < count // NS)
        def _():
            @pl.loop(0, NS // 2)
            def _(s):
                n = s * (count // NS) + j

                @pl.when(n == 0)
                def _():
                    start_pages(src, dst, sem, pl.ds(count * BLOCK - LEAD, LEAD), 4)
                    start_pages(src, dst, sem, pl.ds(0, BLOCK - LEAD), 4)

                @pl.when(n > 0)
                def _():
                    start_pages(src, dst, sem, pl.ds(n * BLOCK - LEAD, BLOCK), 4)

                start_pages(src, dst, sem, pl.ds((n + count // 2) * BLOCK - LEAD, BLOCK), 2)

    def start_keys(cache, slot, runs):
        src, ring, sem, order = cache
        for s, swap in (divmod(n, 2) for n in order):
            for queue in range(2):
                pair = 2 * (queue ^ swap)
                for j, row, count in runs:
                    at = j * (KEYS // 4) + (s * STEPS * KEYS + row - OLD) // 4
                    pltpu.make_async_copy(
                        src.at[pl.ds(at, count // 4), pl.ds(pair, 2)],
                        ring.at[slot, s // 2, pl.ds(row // 4, count // 4),
                                pl.ds(s % 2 * 4 + pair, 2)],
                        sem.at[slot]).start(priority=queue)

    def start_block(cache, j):
        start_keys(cache, j % DEPTH, ((j, 0, KEYS),))

    def slab(w, n, cols):
        return w.at[pl.ds(n * (cols // PAGE), cols // PAGE)]

    def times(lhs, rows):
        bands = rows[...].reshape(16, -1, PAGE, 128)
        return jnp.stack([
            jnp.dot(lhs.astype(BF16), bands[:, c, r:r + 8].reshape(128, 128),
                    preferred_element_type=F32)
            for c in range(bands.shape[1]) for r in range(0, PAGE, 8)])

    def per_entry(lhs, fn):
        halves = []
        for half in range(NS // M):
            part = lhs[half * M:(half + 1) * M].astype(BF16)
            parts = [fn(part, 2 * b + half) for b in range(B)]
            batch = jax.lax.broadcasted_iota(jnp.int32, parts[0].shape, 0) % B
            merged = parts[0]
            for b in range(1, B):
                merged = jnp.where(batch == b, parts[b], merged)
            halves.append(merged)
        return jnp.concatenate(halves, axis=0)

    def scores(i, slot, lo, hi):
        s = per_entry(qs[i], lambda q, p: jax.lax.dot_general(
            q, k_ring[slot, p, 0:hi // 4].reshape(2 * hi, DH), (((1,), (1,)), ((), ())),
            preferred_element_type=F32)) * (DH ** -0.5)
        row, key = (jax.lax.broadcasted_iota(jnp.int32, s.shape, d) for d in range(2))
        return jnp.where(jnp.logical_and(((row ^ key) & 4) == 0, key >= 2 * lo), s, -jnp.inf)

    def softmax_step(i, s):
        old = run_max[i]
        new = jnp.maximum(old, jnp.max(s, axis=-1, keepdims=True))
        p = jnp.exp(s - new[:, 0:1])
        scale = jnp.exp(old - new)
        run_max[i] = new
        run_sum[i] = scale * run_sum[i] + jnp.sum(p, axis=-1, keepdims=True)
        run_pv[i] = scale * run_pv[i]
        return p

    def accumulate(i, slot, p):
        rows = p.shape[1]
        run_pv[i] += per_entry(p, lambda w, e: jnp.dot(
            w, v_ring[slot, e, 0:rows // 8].reshape(rows, DH), preferred_element_type=F32))

    def hidden(n):
        g = g_acc[n]
        return (g * jax.nn.sigmoid(g)) * u_acc[n]

    def project(i):
        heads = run_pv[i] / run_sum[i]
        total = a_acc[...]
        for c in range(H // HS):
            rows = heads[c // 2 * M:(c // 2 + 1) * M]
            if c % 2:
                rows = pltpu.roll(rows, B, 0)
            total += times(rows, slab(wo, HS * c + i, D))
        a_acc[...] = total

    pl.loop(0, N_A // NS)(lambda j: start_weights(wq_hbm, wq, w_sem.at[0], N_A, j))
    small = [pltpu.make_async_copy(src, dst, small_sem)
             for src, dst in ((x_hbm, x_in), (wr_hbm, wr), (gw_hbm, gw))]
    for copy in small:
        copy.start()
    pl.loop(0, N_F // NS)(lambda j: start_weights(wg_hbm, wg, w_sem.at[1], N_F, j))
    for copy in small:
        copy.wait()

    x = x_in[...].astype(F32)
    x = jnp.concatenate([x, x], axis=0)
    for n in range(D // 128):
        xs[n] = x[:, n * 128:(n + 1) * 128]
    for w, dst in ((gw, gate), (wr, router)):
        logit = jnp.sum(x * w[...].astype(F32).reshape(1, D), axis=-1, keepdims=True)
        dst[...] = jnp.broadcast_to(jax.nn.sigmoid(logit), dst.shape)
    for acc in (q_acc, g_acc, u_acc, y_acc, a_acc, run_sum, run_pv):
        acc[...] = jnp.zeros(acc.shape, F32)
    run_max[...] = jnp.full(run_max.shape, LOWEST, F32)

    for n, (w, acc, arriving) in enumerate((
            (wq, q_acc, (wu_hbm, wu, w_sem.at[2], N_F)),
            (wg, g_acc, (wo_hbm, wo, w_sem.at[3], N_A)),
            (wu, u_acc, (wd_hbm, wd, w_sem.at[4], N_D)))):
        wait_all(w, w_sem.at[n])

        @pl.loop(0, D // 128)
        def _(j):
            start_weights(*arriving, j)
            acc[...] += times(xs[j], slab(w, j, acc.shape[0] * 128))

    upper = jax.lax.broadcasted_iota(jnp.int32, (HS, M, DH), 1) >= B
    for half in range(NS // M):
        h0 = 2 * half * HS
        qs[:, half * M:(half + 1) * M] = jnp.where(
            upper, q_acc[h0 + HS:h0 + 2 * HS], q_acc[h0:h0 + HS])

    keys, values = (k_hbm, k_ring, k_sem, K_ORDER), (v_hbm, v_ring, v_sem, V_ORDER)
    for cache in (keys, values):
        start_keys(cache, 0, ((STEPS, 0, OLD), (0, OLD, KEYS - OLD)))
    for j in range(1, DEPTH):
        start_block(keys, j)
        start_block(values, j)
    wait_all(wo, w_sem.at[3])
    wait_all(wd.at[pl.ds(0, N_D * BLOCK)], w_sem.at[4])

    @pl.loop(0, STEPS)
    def _(j):
        i, slot, first = j // JH, j % DEPTH, j % JH == 0
        before = (i + HS - 1) % HS

        wait_all(k_ring.at[slot], k_sem.at[slot])
        p = softmax_step(i, scores(i, slot, jnp.where(first, OLD, 0), KEYS))

        @pl.when(first)
        def _():
            p_old[...] = softmax_step(before, scores(before, slot, 0, OLD))

        @pl.when(j + DEPTH < STEPS)
        def _():
            start_block(keys, j + DEPTH)

        @pl.when(j + DEPTH == STEPS)
        def _():
            @pl.loop(0, TAIL * SLAB)
            def _(n):
                start_pages(wd_hbm, wd, tail_sem.at[n // SLAB],
                            pl.ds((N_D + n) * BLOCK, BLOCK), 4)

        wait_all(v_ring.at[slot], v_sem.at[slot])
        accumulate(i, slot, p)

        @pl.when(first)
        def _():
            accumulate(before, slot, p_old[...])

        @pl.when(j + DEPTH < STEPS)
        def _():
            start_block(values, j + DEPTH)

        @pl.when(j < N_D // SLAB)
        def _():
            y_acc[...] += times(hidden(j), slab(wd, j, D))

        last = j == STEPS - 1

        @pl.when(jnp.logical_or(jnp.logical_and(first, j > 0), last))
        def _():
            project(jnp.where(last, i, before))

    @pl.loop(0, TAIL, init_carry=y_acc[...])
    def y(n, total):
        lhs, rows = hidden(N_D // SLAB + n), slab(wd, N_D // SLAB + n, D)
        wait_all(rows, tail_sem.at[n])
        return total + times(lhs, rows)

    x, g = xs[...], gate[...]
    out = g * a_acc[...] + (1.0 - g) * (x + (x * 0.0 + y * router[...]))
    out = jnp.concatenate([out[n] for n in range(D // 128)], axis=1)
    out_ref[...] = out[0:B, :].astype(out_ref.dtype)


def _pages(w):
    r, c = w.shape
    return w.reshape(r // 8, 8, c // 128, 128).transpose(0, 2, 1, 3).reshape(-1, PAGE, 128)


@jax.jit
def pallas_gated_mix__mha_block_cached__moe_arch_mod__decode_kernel(
    A_x: jax.Array,
    A_k_cache: jax.Array,
    A_v_cache: jax.Array,
    A_wq: jax.Array,
    A_wo: jax.Array,
    B_x: jax.Array,
    B_w_r: jax.Array,
    B_w_gate: jax.Array,
    B_w_up: jax.Array,
    B_w_down: jax.Array,
    gate_w: jax.Array,
):
    del B_x
    dma_sem = pltpu.SemaphoreType.DMA

    def resident(blocks):
        return pltpu.VMEM((blocks * BLOCK, PAGE, 128), BF16)

    def tiles(cols):
        return pltpu.VMEM((cols // 128, M, 128), F32)

    out = pl.pallas_call(
        _kernel,
        out_shape=jax.ShapeDtypeStruct((B, D), BF16),
        in_specs=[pl.BlockSpec(memory_space=pl.ANY)] * 10,
        out_specs=pl.BlockSpec(memory_space=pltpu.VMEM),
        scratch_shapes=[
            pltpu.VMEM((DEPTH, NS // 2, KEYS // 4, 8, DH), BF16),
            pltpu.VMEM((DEPTH, NS // 2, KEYS // 4, 8, DH), BF16),
            resident(N_A),
            resident(N_A),
            resident(N_F),
            resident(N_F),
            resident(N_F),
            pltpu.VMEM((B, D), BF16),
            pltpu.VMEM((D,), BF16),
            pltpu.VMEM((D,), BF16),
            tiles(D),
            pltpu.VMEM((M, 128), F32),
            pltpu.VMEM((M, 128), F32),
            tiles(H * DH),
            tiles(F),
            tiles(F),
            tiles(D),
            tiles(D),
            pltpu.VMEM((HS, NS, DH), F32),
            pltpu.VMEM((HS, NS, 128), F32),
            pltpu.VMEM((HS, NS, 128), F32),
            pltpu.VMEM((HS, NS, DH), F32),
            pltpu.VMEM((NS, 2 * OLD), F32),
            dma_sem((DEPTH,)),
            dma_sem((DEPTH,)),
            dma_sem((5,)),
            dma_sem((TAIL,)),
            dma_sem,
        ],
        compiler_params=pltpu.CompilerParams(
            vmem_limit_bytes=64 * 1024 * 1024,
            disable_bounds_checks=True,
            disable_semaphore_checks=True,
        ),
    )(A_x.reshape(B, D), A_k_cache.reshape(-1, 4, DH), A_v_cache.reshape(-1, 4, DH),
      _pages(A_wq), _pages(A_wo), B_w_r, _pages(B_w_gate), _pages(B_w_up), _pages(B_w_down),
      gate_w)
    return out.reshape(B, 1, D)
```

```python
import jax
import jax.experimental.pallas as pl
import jax.experimental.pallas.tpu as pltpu
import jax.numpy as jnp
import numpy as np

B, D, H, SK, DH, F = 4, 1024, 32, 8192, 128, 3584

M = 8
KEYS = 256
OLD = KEYS // 4
PAGE = 32
BLOCK, LEAD = KEYS // PAGE, OLD // PAGE
NS = 16
HS = B * H // NS
JH = SK // KEYS
STEPS = HS * JH
DEPTH = 2
N_F = D * F // (KEYS * 128)
N_A = D * H * DH // (KEYS * 128)
SLAB = 128 * D // (KEYS * 128)
TAIL = 4
N_D = N_F - TAIL * SLAB
assert N_F % NS == 0 and N_D % NS == 0 and N_A // NS <= D // 128 and N_D // SLAB < STEPS

K_ORDER = (0, 8, 25, 17, 21, 29, 12, 4, 10, 2, 26, 7, 19, 23, 31, 14)
V_ORDER = (2, 6, 14, 12, 29, 21, 19, 27, 10, 4, 0, 16, 24, 9, 22, 30)
assert all(sorted(n // 2 for n in order) == list(range(NS)) for order in (K_ORDER, V_ORDER))

F32, BF16 = jnp.float32, jnp.bfloat16
LOWEST = float(np.finfo(np.float32).min)


def _kernel(x_hbm, k_hbm, v_hbm, wq_hbm, wo_hbm, wr_hbm, wg_hbm, wu_hbm, wd_hbm, gw_hbm,
            out_ref,
            k_ring, v_ring, wq, wo, wg, wu, wd, x_in, wr, gw,
            xs, gate, router, q_acc, g_acc, u_acc, y_acc, a_acc,
            qs, run_max, run_sum, run_pv, p_old,
            k_sem, v_sem, w_sem, tail_sem, small_sem):

    def wait_all(buf, sem):
        pltpu.make_async_copy(buf, buf, sem).wait()

    def start_pages(src, dst, sem, pages, fast):
        for queue, rows in enumerate((pl.ds(0, fast), pl.ds(fast, PAGE - fast))):
            pltpu.make_async_copy(
                src.at[pages, rows], dst.at[pages, rows], sem).start(priority=queue)

    def start_weights(src, dst, sem, count, j):
        @pl.when(j < count // NS)
        def _():
            @pl.loop(0, NS // 2)
            def _(s):
                n = s * (count // NS) + j

                @pl.when(n == 0)
                def _():
                    start_pages(src, dst, sem, pl.ds(count * BLOCK - LEAD, LEAD), 4)
                    start_pages(src, dst, sem, pl.ds(0, BLOCK - LEAD), 4)

                @pl.when(n > 0)
                def _():
                    start_pages(src, dst, sem, pl.ds(n * BLOCK - LEAD, BLOCK), 4)

                start_pages(src, dst, sem, pl.ds((n + count // 2) * BLOCK - LEAD, BLOCK), 2)

    def start_keys(cache, slot, runs):
        src, ring, sem, order = cache
        for s, swap in (divmod(n, 2) for n in order):
            for queue in range(2):
                pair = 2 * (queue ^ swap)
                for j, row, count in runs:
                    at = j * (KEYS // 4) + (s * STEPS * KEYS + row - OLD) // 4
                    pltpu.make_async_copy(
                        src.at[pl.ds(at, count // 4), pl.ds(pair, 2)],
                        ring.at[slot, s // 2, pl.ds(row // 4, count // 4),
                                pl.ds(s % 2 * 4 + pair, 2)],
                        sem.at[slot]).start(priority=queue)

    def start_block(cache, j):
        start_keys(cache, j % DEPTH, ((j, 0, KEYS),))

    def slab(w, n, cols):
        return w.at[pl.ds(n * (cols // PAGE), cols // PAGE)]

    def times(lhs, rows):
        bands = rows[...].reshape(16, -1, PAGE, 128)
        return jnp.stack([
            jnp.dot(lhs.astype(BF16), bands[:, c, r:r + 8].reshape(128, 128),
                    preferred_element_type=F32)
            for c in range(bands.shape[1]) for r in range(0, PAGE, 8)])

    def per_entry(lhs, fn):
        halves = []
        for half in range(NS // M):
            part = lhs[half * M:(half + 1) * M].astype(BF16)
            parts = [fn(part, 2 * b + half) for b in range(B)]
            batch = jax.lax.broadcasted_iota(jnp.int32, parts[0].shape, 0) % B
            merged = parts[0]
            for b in range(1, B):
                merged = jnp.where(batch == b, parts[b], merged)
            halves.append(merged)
        return jnp.concatenate(halves, axis=0)

    def scores(i, slot, lo, hi):
        s = per_entry(qs[i], lambda q, p: jax.lax.dot_general(
            q, k_ring[slot, p, 0:hi // 4].reshape(2 * hi, DH), (((1,), (1,)), ((), ())),
            preferred_element_type=F32)) * (DH ** -0.5)
        row, key = (jax.lax.broadcasted_iota(jnp.int32, s.shape, d) for d in range(2))
        return jnp.where(jnp.logical_and(((row ^ key) & 4) == 0, key >= 2 * lo), s, -jnp.inf)

    def softmax_step(i, s):
        old = run_max[i]
        new = jnp.maximum(old, jnp.max(s, axis=-1, keepdims=True))
        p = jnp.exp(s - new[:, 0:1])
        scale = jnp.exp(old - new)
        run_max[i] = new
        run_sum[i] = scale * run_sum[i] + jnp.sum(p, axis=-1, keepdims=True)
        run_pv[i] = scale * run_pv[i]
        return p

    def accumulate(i, slot, p):
        rows = p.shape[1]
        run_pv[i] += per_entry(p, lambda w, e: jnp.dot(
            w, v_ring[slot, e, 0:rows // 8].reshape(rows, DH), preferred_element_type=F32))

    def hidden(n):
        g = g_acc[n]
        return (g * jax.nn.sigmoid(g)) * u_acc[n]

    def project(i):
        heads = run_pv[i] / run_sum[i]
        total = a_acc[...]
        for c in range(H // HS):
            rows = heads[c // 2 * M:(c // 2 + 1) * M]
            if c % 2:
                rows = pltpu.roll(rows, B, 0)
            total += times(rows, slab(wo, HS * c + i, D))
        a_acc[...] = total

    pl.loop(0, N_A // NS)(lambda j: start_weights(wq_hbm, wq, w_sem.at[0], N_A, j))
    small = [pltpu.make_async_copy(src, dst, small_sem)
             for src, dst in ((x_hbm, x_in), (wr_hbm, wr), (gw_hbm, gw))]
    for copy in small:
        copy.start()
    pl.loop(0, N_F // NS)(lambda j: start_weights(wg_hbm, wg, w_sem.at[1], N_F, j))
    for copy in small:
        copy.wait()

    x = x_in[...].astype(F32)
    x = jnp.concatenate([x, x], axis=0)
    for n in range(D // 128):
        xs[n] = x[:, n * 128:(n + 1) * 128]
    for w, dst in ((gw, gate), (wr, router)):
        logit = jnp.sum(x * w[...].astype(F32).reshape(1, D), axis=-1, keepdims=True)
        dst[...] = jnp.broadcast_to(jax.nn.sigmoid(logit), dst.shape)
    for acc in (q_acc, g_acc, u_acc, y_acc, a_acc, run_sum, run_pv):
        acc[...] = jnp.zeros(acc.shape, F32)
    run_max[...] = jnp.full(run_max.shape, LOWEST, F32)

    for n, (w, acc, arriving) in enumerate((
            (wq, q_acc, (wu_hbm, wu, w_sem.at[2], N_F)),
            (wg, g_acc, (wo_hbm, wo, w_sem.at[3], N_A)),
            (wu, u_acc, (wd_hbm, wd, w_sem.at[4], N_D)))):
        wait_all(w, w_sem.at[n])

        @pl.loop(0, D // 128)
        def _(j):
            start_weights(*arriving, j)
            acc[...] += times(xs[j], slab(w, j, acc.shape[0] * 128))

    upper = jax.lax.broadcasted_iota(jnp.int32, (HS, M, DH), 1) >= B
    for half in range(NS // M):
        h0 = 2 * half * HS
        qs[:, half * M:(half + 1) * M] = jnp.where(
            upper, q_acc[h0 + HS:h0 + 2 * HS], q_acc[h0:h0 + HS])

    keys, values = (k_hbm, k_ring, k_sem, K_ORDER), (v_hbm, v_ring, v_sem, V_ORDER)

    @pl.loop(0, 2 * DEPTH)
    def _(n):
        for c, cache in enumerate((keys, values)):
            @pl.when(n == c)
            def _():
                start_keys(cache, 0, ((STEPS, 0, OLD), (0, OLD, KEYS - OLD)))

            @pl.when(jnp.logical_and(n > c, n % 2 == c))
            def _():
                start_block(cache, n // 2)

    wait_all(wo, w_sem.at[3])
    wait_all(wd.at[pl.ds(0, N_D * BLOCK)], w_sem.at[4])

    @pl.loop(0, STEPS)
    def _(j):
        i, slot, first = j // JH, j % DEPTH, j % JH == 0
        before = (i + HS - 1) % HS

        wait_all(k_ring.at[slot], k_sem.at[slot])
        p = softmax_step(i, scores(i, slot, jnp.where(first, OLD, 0), KEYS))

        @pl.when(first)
        def _():
            p_old[...] = softmax_step(before, scores(before, slot, 0, OLD))

        @pl.when(j + DEPTH < STEPS)
        def _():
            start_block(keys, j + DEPTH)

        @pl.when(j + DEPTH == STEPS)
        def _():
            @pl.loop(0, TAIL * SLAB)
            def _(n):
                start_pages(wd_hbm, wd, tail_sem.at[n // SLAB],
                            pl.ds((N_D + n) * BLOCK, BLOCK), 2)

        wait_all(v_ring.at[slot], v_sem.at[slot])
        accumulate(i, slot, p)

        @pl.when(first)
        def _():
            accumulate(before, slot, p_old[...])

        @pl.when(j + DEPTH < STEPS)
        def _():
            start_block(values, j + DEPTH)

        @pl.when(j < N_D // SLAB)
        def _():
            y_acc[...] += times(hidden(j), slab(wd, j, D))

        last = j == STEPS - 1

        @pl.when(jnp.logical_or(jnp.logical_and(first, j > 0), last))
        def _():
            project(jnp.where(last, i, before))

    x, g, r = xs[...], gate[...], router[...]
    known = g * a_acc[...] + (1.0 - g) * (x + (x * 0.0 + y_acc[...] * r))

    @pl.loop(0, TAIL, init_carry=known)
    def out(n, total):
        lhs, rows = hidden(N_D // SLAB + n), slab(wd, N_D // SLAB + n, D)
        wait_all(rows, tail_sem.at[n])
        return total + ((1.0 - g) * r) * times(lhs, rows)

    out = jnp.concatenate([out[n] for n in range(D // 128)], axis=1)
    out_ref[...] = out[0:B, :].astype(out_ref.dtype)


def _pages(w):
    r, c = w.shape
    return w.reshape(r // 8, 8, c // 128, 128).transpose(0, 2, 1, 3).reshape(-1, PAGE, 128)


@jax.jit
def pallas_gated_mix__mha_block_cached__moe_arch_mod__decode_kernel(
    A_x: jax.Array,
    A_k_cache: jax.Array,
    A_v_cache: jax.Array,
    A_wq: jax.Array,
    A_wo: jax.Array,
    B_x: jax.Array,
    B_w_r: jax.Array,
    B_w_gate: jax.Array,
    B_w_up: jax.Array,
    B_w_down: jax.Array,
    gate_w: jax.Array,
):
    del B_x
    dma_sem = pltpu.SemaphoreType.DMA

    def resident(blocks):
        return pltpu.VMEM((blocks * BLOCK, PAGE, 128), BF16)

    def tiles(cols):
        return pltpu.VMEM((cols // 128, M, 128), F32)

    out = pl.pallas_call(
        _kernel,
        out_shape=jax.ShapeDtypeStruct((B, D), BF16),
        in_specs=[pl.BlockSpec(memory_space=pl.ANY)] * 10,
        out_specs=pl.BlockSpec(memory_space=pltpu.VMEM),
        scratch_shapes=[
            pltpu.VMEM((DEPTH, NS // 2, KEYS // 4, 8, DH), BF16),
            pltpu.VMEM((DEPTH, NS // 2, KEYS // 4, 8, DH), BF16),
            resident(N_A),
            resident(N_A),
            resident(N_F),
            resident(N_F),
            resident(N_F),
            pltpu.VMEM((B, D), BF16),
            pltpu.VMEM((D,), BF16),
            pltpu.VMEM((D,), BF16),
            tiles(D),
            pltpu.VMEM((M, 128), F32),
            pltpu.VMEM((M, 128), F32),
            tiles(H * DH),
            tiles(F),
            tiles(F),
            tiles(D),
            tiles(D),
            pltpu.VMEM((HS, NS, DH), F32),
            pltpu.VMEM((HS, NS, 128), F32),
            pltpu.VMEM((HS, NS, 128), F32),
            pltpu.VMEM((HS, NS, DH), F32),
            pltpu.VMEM((NS, 2 * OLD), F32),
            dma_sem((DEPTH,)),
            dma_sem((DEPTH,)),
            dma_sem((5,)),
            dma_sem((TAIL,)),
            dma_sem,
        ],
        compiler_params=pltpu.CompilerParams(
            vmem_limit_bytes=64 * 1024 * 1024,
            disable_bounds_checks=True,
            disable_semaphore_checks=True,
        ),
    )(A_x.reshape(B, D), A_k_cache.reshape(-1, 4, DH), A_v_cache.reshape(-1, 4, DH),
      _pages(A_wq), _pages(A_wo), B_w_r, _pages(B_w_gate), _pages(B_w_up), _pages(B_w_down),
      gate_w)
    return out.reshape(B, 1, D)
```
